```python
import jax
import jax.numpy as jnp

def _softmax(x, axis=-1):
    return jax.nn.softmax(x, axis=axis)
def _gelu(x):
    return jax.nn.gelu(x, approximate=True)
def _silu(x):
    return jax.nn.silu(x)
def _sigmoid(x):
    return jax.nn.sigmoid(x)
def _layernorm(x, axis=-1, eps=1e-5):
    m = jnp.mean(x, axis=axis, keepdims=True)
    v = jnp.var(x, axis=axis, keepdims=True)
    return (x - m) / jnp.sqrt(v + eps)
def _scatter_add(tgt, idx, src, axis=0):
    return tgt.at[idx].add(src)
def _segment_sum(src, seg, n):
    return jax.ops.segment_sum(src, seg, n)
class _Rng:
    def __init__(self, key):
        self._k = key
    def _next(self):
        self._k, sub = jax.random.split(self._k)
        return sub
    def normal(self, shape):
        return jax.random.normal(self._next(), shape, dtype=jnp.bfloat16)
    def randint(self, lo, hi, shape):
        return jax.random.randint(self._next(), shape, lo, hi, dtype=jnp.int32)
    def uniform(self, shape, lo=0.0, hi=1.0):
        return jax.random.uniform(self._next(), shape, jnp.bfloat16, lo, hi)
    def permutation(self, n):
        return jax.random.permutation(self._next(), n)


kernel_name = 'gated_mix__sliding_block_cached__moe_arch_mod__decode'

def setup_inputs():
    _rng = _Rng(jax.random.key(int.from_bytes(__import__("os").urandom(4), "little")))
    _w = (lambda a: (lambda t: t.astype(jnp.bfloat16) if jnp.issubdtype(t.dtype, jnp.floating) else t)(jnp.asarray(a)))
    def _A_setup():
        B, Sq, D = 1, 1, 640
        Hq, Hkv, Sk, Dh = 32, 32, 32768, 192
        assert Hq % Hkv == 0, (Hq, Hkv)
        return {
            "x": _w((lambda *s: _rng.normal(s) * 0.05)(B, Sq, D)),
            "k_cache": _w((lambda *s: _rng.normal(s) * 0.05)(B, Hkv, Sk, Dh)),
            "v_cache": _w((lambda *s: _rng.normal(s) * 0.05)(B, Hkv, Sk, Dh)),
            "wq": _w((lambda *s: _rng.normal(s) * 0.05)(D, Hq * Dh) * (D ** -0.5)),
            "wo": _w((lambda *s: _rng.normal(s) * 0.05)(Hq * Dh, D) * ((Hq * Dh) ** -0.5)),
        }
    _A_in = _A_setup()

    def _B_setup():
        B, S, D, F, C = 1, 1, 640, 1536, 1
        return {
            "x": _w((lambda *s: _rng.normal(s) * 0.05)(B, S, D)),
            "w_r": _w((lambda *s: _rng.normal(s) * 0.05)(D)),
            "w_gate": _w((lambda *s: _rng.normal(s) * 0.05)(D, F)),
            "w_up": _w((lambda *s: _rng.normal(s) * 0.05)(D, F)),
            "w_down": _w((lambda *s: _rng.normal(s) * 0.05)(F, D)),
        }
    _B_in = _B_setup()

    return {
        "A_x": _A_in["x"],
        "A_k_cache": _A_in["k_cache"],
        "A_v_cache": _A_in["v_cache"],
        "A_wq": _A_in["wq"],
        "A_wo": _A_in["wo"],
        "B_x": _B_in["x"],
        "B_w_r": _B_in["w_r"],
        "B_w_gate": _B_in["w_gate"],
        "B_w_up": _B_in["w_up"],
        "B_w_down": _B_in["w_down"],
        "gate_w": _w((lambda *s: _rng.normal(s) * 0.05)(640)),
    }

def reference(A_x, A_k_cache, A_v_cache, A_wq, A_wo, B_x, B_w_r, B_w_gate, B_w_up, B_w_down, gate_w):
    def _A_ref(x, k_cache, v_cache, wq, wo):
        B, Sq, D = x.shape
        Hq, Dh = 32, 192
        Hkv, Sk = k_cache.shape[1], k_cache.shape[2]
        W = min(4096, max(256, Sk // 4))
        rep = Hq // Hkv
        q = (lambda x, *d: x.transpose(*d))((x @ wq).reshape(B, Sq, Hq, Dh), 0, 2, 1, 3)
        k = jnp.repeat(k_cache[:, :, Sk - W:, :], rep, axis=1)
        v = jnp.repeat(v_cache[:, :, Sk - W:, :], rep, axis=1)
        scores = jnp.einsum("bhqd,bhkd->bhqk", q, k) * (Dh ** -0.5)
        p = _softmax(scores, axis=-1)
        o = jnp.einsum("bhqk,bhkd->bhqd", p, v)
        return (lambda x, *d: x.transpose(*d))(o, 0, 2, 1, 3).reshape(B, Sq, Hq * Dh) @ wo

    def _B_ref(x, w_r, w_gate, w_up, w_down):
        B, S, D = x.shape
        C = 1
        r = x @ w_r
        idx = jnp.argsort(-r, axis=-1)[:, :C]
        idx_e = jnp.repeat(idx.reshape(B, C, 1), D, axis=2)
        x_sel = jnp.take_along_axis(x, idx_e, axis=1)
        g = _silu(x_sel @ w_gate)
        u = x_sel @ w_up
        y = (g * u) @ w_down
        r_sel = _sigmoid(jnp.take_along_axis(r, idx, axis=1))
        y = y * r_sel.reshape(B, C, 1)
        b_off = (jnp.arange(B) * S).reshape(B, 1)
        flat_idx = (idx + b_off).reshape(B * C)
        zero = (x * 0.0).reshape(B * S, D)
        upd = _scatter_add(zero, flat_idx, y.reshape(B * C, D), axis=0)
        return x + upd.reshape(B, S, D)

    x = A_x
    g = _sigmoid((x * gate_w).sum(-1, keepdims=True))
    a = _A_ref(x, A_k_cache, A_v_cache, A_wq, A_wo)
    b = _B_ref(x, B_w_r, B_w_gate, B_w_up, B_w_down)
    return g * a + (1 - g) * b
```

```python
import jax
import jax.numpy as jnp
import jax.experimental.pallas as pl
import jax.experimental.pallas.tpu as pltpu

H, DH, SK, D, F = 32, 192, 32768, 640, 1536
W = min(4096, max(256, SK // 4))
BASE = SK - W
M = 8

NS, HS = 64, 32
KG, KC = 3, 1024
NG = DH // 16
WB = 512
LG = 46
LE = 44
TW = 15
TAIL, TAIL0 = (4,) * 14, 8

f32, bf16 = jnp.float32, jnp.bfloat16


def _every(t0, n, d):
    return [t0 + j * d for j in range(n)]


def _by_step(tasks):
    by = {}
    for t, fn in tasks:
        by.setdefault(t, []).append(fn)
    return by


def _kernel(x_hbm, kT, vT, wq, wo, wr_hbm, wg, wu, wd, gw_hbm, out_ref,
            x_v, wr_v, gw_v, k_b, v_b, wc_b, wo_b, wd_b, pr_s, o_s, s_s, p_s, a_s, hb_s,
            kv_sem, w_sem, t_sem, s_sem):
    def kv_copy(which, h, j, slot):
        src = (kT, vT)[which].at[h]
        buf = k_b.at[h & 3] if which == 0 else v_b.at[h & 1]
        par, j = divmod(j, HS // 2)
        c, r = divmod(j, NG // KG)
        groups, rows = pl.ds(r * KG, KG), pl.ds(8 * par, 8)
        return pltpu.make_async_copy(src.at[groups, rows, pl.ds(BASE + c * KC, KC)],
                                     buf.at[groups, rows, pl.ds(c * KC, KC)], kv_sem.at[slot])

    def kv_wait(slot):
        kv_copy(0, 0, 0, slot).wait()

    def last_piece_of(col):
        return HS // 2 + (NG // KG) * (col // KC) - 1

    def col_pieces(src, blk, i, s):
        tiles = D // 8
        n = 16 if src is wq else 4
        cols = pl.ds(pl.multiple_of(blk * WB, WB), WB)
        out = []
        for j in range((s * tiles) // NS, ((s + 1) * tiles) // NS):
            rows = pl.ds(8 * ((j % n) * (tiles // n) + j // n), 8)
            out.append(pltpu.make_async_copy(src.at[rows, cols], wc_b.at[i & 1, rows], w_sem.at[i & 1]))
        return out

    def wo_pieces(blk, i, s):
        rows = pl.ds(pl.multiple_of((s % 2) * (H * DH // 2) + blk * (WB // 2) + 8 * (s // 2), 8), 8)
        return [pltpu.make_async_copy(wo.at[rows], wo_b.at[rows], w_sem.at[i & 1])]

    def wd_copy(r0, n, sem):
        return pltpu.make_async_copy(wd.at[pl.ds(r0, n)], wd_b.at[pl.ds(r0, n)], sem)

    def slab_wait(i):
        pltpu.make_async_copy(wc_b.at[0], wc_b.at[0], w_sem.at[i & 1]).wait()

    small = [pltpu.make_async_copy(x_hbm, x_v, s_sem.at[0]),
             pltpu.make_async_copy(gw_hbm, gw_v, s_sem.at[1]),
             pltpu.make_async_copy(wr_hbm, wr_v, s_sem.at[2])]

    def kv_tile(buf, sl):
        t = buf[:, :, sl]
        return t.reshape(DH, t.shape[-1])

    def qk_tasks(h, t_qk, t_sm):
        st = {}
        cw = W // len(t_qk)

        def qk(j):
            def fn():
                if j == 0:
                    t0 = (3 * h) >> 1
                    q2 = jnp.concatenate([pr_s[t0], pr_s[t0 + 1]], axis=1)
                    if isinstance(h, int):
                        q = q2[:, 64 * (h % 2):64 * (h % 2) + DH]
                    else:
                        q = jnp.where((h & 1) == 0, q2[:, :DH], q2[:, 64:])
                    st["q"] = q.astype(bf16)
                sl = slice(j * cw, (j + 1) * cw)
                s_s[:, sl] = jnp.dot(st["q"], kv_tile(k_b.at[h & 3], sl),
                                     preferred_element_type=f32) * (DH ** -0.5)
            return fn

        def sm_max():
            st["m"] = jnp.max(s_s[...], axis=-1, keepdims=True)

        def sm_exp():
            e = jnp.exp(s_s[...] - st["m"])
            s_s[...] = e
            st["l"] = jnp.sum(e, axis=-1, keepdims=True)

        def sm_norm():
            p_s[h & 1] = s_s[...] * (1.0 / st["l"])

        return [(t, qk(j)) for j, t in enumerate(t_qk)] + list(zip(t_sm, (sm_max, sm_exp, sm_norm)))

    def pv_tasks(h, t_pv):
        st = {}
        cw = W // len(t_pv)

        def pv(j):
            def fn():
                sl = slice(j * cw, (j + 1) * cw)
                part = jax.lax.dot_general(p_s[h & 1, :, sl].astype(bf16), kv_tile(v_b.at[h & 1], sl),
                                           (((1,), (1,)), ((), ())), preferred_element_type=f32)
                st["o"] = part if j == 0 else st["o"] + part
                if j == len(t_pv) - 1:
                    o_s[h] = st["o"]
            return fn

        return [(t, pv(j)) for j, t in enumerate(t_pv)]

    def proj_tasks(i):
        def proj(j):
            def fn():
                pr_s[4 * i + j] = jnp.dot(jnp.broadcast_to(x_v[0], (M, D)), wc_b[i & 1, :, j * 128:(j + 1) * 128],
                                          preferred_element_type=f32)
            return fn

        return [(TW + 2 * j, proj(j)) for j in range(WB // 128)]

    def o_task(hd):
        def fn():
            rows = pl.ds(pl.multiple_of(hd * DH, 64), DH)
            a_s[...] += jnp.dot(o_s[hd].astype(bf16), wo_b[rows, :], preferred_element_type=f32)
        return fn

    def std_qk(h):
        return qk_tasks(h, _every(TW + 8, 8, 2), _every(TW + 24, 3, 2))

    def std_pv(h):
        return pv_tasks(h, _every(LG, 8, 2))

    def stream_round(i, w_pieces, tasks, first=False):
        by = _by_step(tasks)
        assert max(by, default=0) < NS
        for s in range(NS):
            if not first or s - LG >= -HS:
                kv_wait((s - LG) % NS)
            for c in w_pieces(s):
                c.start(priority=0)
            (kv_copy(0, i + 1, s, s) if s < HS else kv_copy(1, i, s - HS, s)).start(priority=1)
            if first and s == 16:
                for c in small:
                    c.start()
            if s == TW and not first:
                slab_wait(i - 1)
            for fn in by.get(s, []):
                fn()

    for j in range(HS):
        kv_copy(0, 0, j, HS + j).start(priority=1)
    stream_round(0, lambda s: col_pieces(wq, 0, 0, s), [], first=True)
    for c in small:
        c.wait()
    a_s[...] = jnp.zeros(a_s.shape, f32)

    for src, i0, lo, hi in ((wq, 0, 1, 12), (wg, 12, 12, 15), (wu, 15, 15, 18)):
        def col_round(i, carry):
            stream_round(i, lambda s: col_pieces(src, i - i0, i, s),
                         proj_tasks(i - 1) + std_qk(i - 1) + std_pv(i - 1))
            return carry
        jax.lax.fori_loop(lo, hi, col_round, 0)

    stream_round(18, lambda s: wo_pieces(0, 18, s),
                 proj_tasks(17) + qk_tasks(17, _every(0, 4, 3), _every(11, 3, 2)) + std_qk(18) + std_pv(17))

    def wo_round(i, carry):
        stream_round(i, lambda s: wo_pieces(i - 18, i, s),
                     [(TW, o_task(i - 19)), (TW + 4, o_task(i - 3))] + std_qk(i) + std_pv(i - 1))
        return carry
    jax.lax.fori_loop(19, 30, wo_round, 0)

    st = {}

    def act():
        g = jnp.concatenate([pr_s[48 + k] for k in range(F // 128)], axis=1)
        u = jnp.concatenate([pr_s[60 + k] for k in range(F // 128)], axis=1)
        st["h"] = (jax.nn.silu(g) * u).astype(bf16)

    def gates():
        xf = x_v[0].astype(f32)
        st["gate"] = jax.nn.sigmoid(jnp.sum(xf * gw_v[...].astype(f32).reshape(1, D), axis=-1, keepdims=True))
        st["rsel"] = jax.nn.sigmoid(jnp.sum(xf * wr_v[...].astype(f32).reshape(1, D), axis=-1, keepdims=True))

    def h_column(j):
        def fn():
            row = st["h"][0:1, WB + 128 * j:WB + 128 * (j + 1)].astype(f32)
            hb_s[128 * j:128 * (j + 1)] = jnp.broadcast_to(row, (128, 128)).T
        return fn

    def down_mxu(r0, r1):
        def fn():
            part = jnp.dot(st["h"][:, r0:r1], wd_b[r0:r1, :], preferred_element_type=f32)
            st["y"] = part + st["y"] if "y" in st else part
        return fn

    def down_vpu(r0, r1):
        for r in range(r0, r1, 8):
            hb = hb_s[r - WB:r - WB + 8]
            part = wd_b[r:r + 8, :].astype(f32) * jnp.concatenate([hb] * (D // 128), axis=1)
            st["z"] = part + st["z"] if "z" in st else part

    stream_round(30, lambda s: [wd_copy(8 * s, 8, w_sem.at[0])],
                 [(0, act), (2, gates)] + [(3 + j, h_column(j)) for j in range((F - WB) // 128)]
                 + [(TW + 2 * j, o_task(11 + j)) for j in range(4)] + std_qk(30) + std_pv(29))

    quarters = [W * (j + 1) // 4 for j in range(4)]
    t_pv30 = [max(last_piece_of(c) + HS + LG - NS, 34 + 3 * j) for j, c in enumerate(quarters)]
    t_pv31 = [last_piece_of(c) + LE for c in quarters]
    by = _by_step([(3 * j, o_task(hd)) for j, hd in enumerate((15, 27, 28, 29))]
                  + qk_tasks(31, _every(LG - HS, 8, 2), _every(LG - HS + 16, 3, 2))
                  + pv_tasks(30, t_pv30) + [(t_pv30[-1] + 3, o_task(30))]
                  + [(t_pv30[-1] + 5, down_mxu(0, WB // 2)), (t_pv30[-1] + 7, down_mxu(WB // 2, WB))]
                  + pv_tasks(31, t_pv31) + [(t_pv31[-1], o_task(31))])
    n0 = WB // 8 + TAIL0
    tail, r = [], WB + 8 * n0
    for n in TAIL:
        tail.append((r, 8 * n))
        r += 8 * n
    assert r == F and n0 % 8 == 0
    n1 = HS + len(tail)
    n_steps = n1 + LE
    assert max(by) < n_steps - 1
    waited, done0 = -LG, 0
    for s in range(n_steps):
        last = s == n_steps - 1
        while done0 < n0 and (last or (s % 8 == 1 and done0 + 8 <= s - TW)):
            wd_copy(WB + 8 * done0, 64, t_sem.at[done0 // 8]).wait()
            down_vpu(WB + 8 * done0, WB + 8 * done0 + 64)
            done0 += 8
        if last:
            xf = x_v[0].astype(f32)
            cb = (1.0 - st["gate"]) * st["rsel"]
            base = st["gate"] * a_s[0:1] + (1.0 - st["gate"]) * (xf + xf * 0.0) + cb * st["y"][0:1]
        while waited <= (s - LG if s < n1 else s - LE):
            if waited < HS:
                kv_wait(waited % NS)
            else:
                r0, n = tail[waited - HS]
                wd_copy(r0, n, t_sem.at[n0 // 8 + waited - HS]).wait()
                down_vpu(r0, r0 + n)
            waited += 1
        if s < n0:
            wd_copy(WB + 8 * s, 8, t_sem.at[s // 8]).start(priority=0)
        if s < HS:
            kv_copy(1, H - 1, s, s).start(priority=1)
        elif s < n1:
            wd_copy(*tail[s - HS], t_sem.at[n0 // 8 + s - HS]).start(priority=1)
        if s == TW:
            slab_wait(30)
        for fn in by.get(s, []):
            fn()
    assert waited == n1 and done0 == n0

    out_ref[0] = (base + cb * jnp.sum(st["z"], axis=0, keepdims=True)).astype(bf16)


@jax.jit
def pallas_gated_mix__sliding_block_cached__moe_arch_mod__decode_kernel(
        A_x, A_k_cache, A_v_cache, A_wq, A_wo, B_x, B_w_r, B_w_gate, B_w_up, B_w_down, gate_w):
    del B_x
    kT = jnp.swapaxes(A_k_cache, 2, 3).reshape(H, NG, 16, SK)
    vT = jnp.swapaxes(A_v_cache, 2, 3).reshape(H, NG, 16, SK)
    vmem, dma = pltpu.VMEM, pltpu.SemaphoreType.DMA
    return pl.pallas_call(
        _kernel,
        out_shape=jax.ShapeDtypeStruct((1, 1, D), bf16),
        in_specs=[pl.BlockSpec(memory_space=pl.ANY)] * 10,
        out_specs=pl.BlockSpec(memory_space=pltpu.VMEM),
        scratch_shapes=[
            vmem((1, 1, D), bf16), vmem((D,), bf16), vmem((D,), bf16),
            vmem((4, NG, 16, W), bf16), vmem((2, NG, 16, W), bf16), vmem((2, D, WB), bf16),
            vmem((H * DH, D), bf16), vmem((F, D), bf16),
            vmem(((H * DH + 2 * F) // 128, M, 128), f32), vmem((H, M, DH), f32),
            vmem((M, W), f32), vmem((2, M, W), f32), vmem((M, D), f32), vmem((F - WB, 128), f32),
            dma((NS,)), dma((2,)), dma((32,)), dma((3,)),
        ],
        compiler_params=pltpu.CompilerParams(
            vmem_limit_bytes=64 * 1024 * 1024,
            disable_semaphore_checks=True,
            disable_bounds_checks=True,
        ),
        name="gated_mix_decode",
    )(A_x, kT, vT, A_wq, A_wo, B_w_r, B_w_gate, B_w_up, B_w_down, gate_w)
```

```python
import jax
import jax.numpy as jnp
import jax.experimental.pallas as pl
import jax.experimental.pallas.tpu as pltpu

H, DH, SK, D, F = 32, 192, 32768, 640, 1536
W = min(4096, max(256, SK // 4))
BASE = SK - W
M = 8

NS, HS = 64, 32
KC = W // 4
QB = 2048
RUN = 32
NT_O, NT_F = H * DH * D // 1024, F * D // 1024
OFF_O, OFF_F = 16, 8
N_HI = 12
LG = 46
TW = 15

f32, bf16 = jnp.float32, jnp.bfloat16


def _sweep(group, quarters):
    firsts = [0, 2, 12, 14, 1, 3, 13, 15]
    return [(r, c) for k in range(0, len(firsts), group) for c in quarters for r in firsts[k:k + group]]


ORDER = (_sweep(2, (0, 1)) + _sweep(2, (2, 3)),
         _sweep(4, (0, 1, 2)) + _sweep(4, (3,)))


def _every(t0, n, d):
    return [t0 + j * d for j in range(n)]


def _by_step(tasks):
    by = {}
    for t, fn in tasks:
        by.setdefault(t, []).append(fn)
    return by


def _kernel(x_hbm, kT, vT, wq, wo, wr_hbm, wg, wu, wd, gw_hbm, out_ref,
            x_v, wr_v, gw_v, k_b, v_b, wq_b, wo_b, gu_b, wd_b, pr_s, o_s, s_s, p_s, a_s, hb_s,
            kv_sem, w_sem, d_sem, p_sem):
    def kv_copy(which, h, j, slot):
        src, buf = (kT, vT)[which].at[h], (k_b, v_b)[which].at[h & 1]
        r, c = ORDER[which][j]
        groups, rows = pl.ds(r // 4, 3), pl.ds(8 * (r % 4), 8)
        return pltpu.make_async_copy(src.at[groups, rows, pl.ds(BASE + c * KC, KC)],
                                     buf.at[groups, rows, pl.ds(c * KC, KC)], kv_sem.at[slot])

    def kv_wait(slot):
        kv_copy(0, 0, 0, slot).wait()

    def tiles_copy(src, dst, t, n, sem):
        return pltpu.make_async_copy(src.at[pl.ds(t, n)], dst.at[pl.ds(t, n)], sem)

    def tiles_wait(n, sem):
        tiles_copy(wo_b, wo_b, 0, n, sem).wait()

    def wq_copy(row_tile, col, n, sem):
        idx = (pl.ds(pl.multiple_of(8 * row_tile, 8), 8), pl.ds(pl.multiple_of(col, 512), n))
        return pltpu.make_async_copy(wq.at[idx], wq_b.at[idx], sem)

    def wq_piece(i, s):
        blk = i // 5 if isinstance(i, int) else jnp.where(i >= 5, 1, 0)
        return wq_copy(5 * (s // 4) + i - 5 * blk, QB * (blk + 1) + 512 * (s % 4), 512, w_sem.at[i & 1])

    def run_piece(src, dst, pos, s, off, sem, may_wrap=False):
        n = src.shape[0]
        run, part = divmod(s, 8)
        t = (run % 2) * (n // 2) + (pos + run // 2) * RUN + 4 * part - off
        if isinstance(t, int):
            t %= n
        elif may_wrap and run == 0 and 4 * part < off:
            t = jnp.where(t < 0, t + n, t)
        return tiles_copy(src, dst, t, 4, sem)

    small = [pltpu.make_async_copy(x_hbm, x_v, p_sem.at[0]),
             pltpu.make_async_copy(gw_hbm, gw_v, p_sem.at[1]),
             pltpu.make_async_copy(wr_hbm, wr_v, p_sem.at[2])]

    def kv_cols(buf, sl):
        t = buf[:, :, sl]
        return t.reshape(DH, t.shape[-1])

    def tile_column(ref, t0, n, stride):
        return jnp.concatenate([ref[t0 + stride * k] for k in range(n)], axis=0)

    def x_rows():
        return jnp.broadcast_to(x_v[0], (M, D))

    def qk_tasks(h, t0):
        st = {}

        def qk(j):
            def fn():
                if j == 0:
                    tile = (3 * h) >> 1
                    q2 = jnp.concatenate([pr_s[tile], pr_s[tile + 1]], axis=1)
                    if isinstance(h, int):
                        q = q2[:, 64 * (h % 2):64 * (h % 2) + DH]
                    else:
                        q = jnp.where((h & 1) == 0, q2[:, :DH], q2[:, 64:])
                    st["q"] = q.astype(bf16)
                sl = slice(j * W // 8, (j + 1) * W // 8)
                s_s[:, sl] = jnp.dot(st["q"], kv_cols(k_b.at[h & 1], sl),
                                     preferred_element_type=f32) * (DH ** -0.5)
            return fn

        def sm_max():
            st["m"] = jnp.max(s_s[...], axis=-1, keepdims=True)

        def sm_exp():
            e = jnp.exp(s_s[...] - st["m"])
            s_s[...] = e
            st["l"] = jnp.sum(e, axis=-1, keepdims=True)

        def sm_norm():
            p_s[h & 1] = s_s[...] * (1.0 / st["l"])

        return list(zip(_every(t0, 11, 2), [qk(j) for j in range(8)] + [sm_max, sm_exp, sm_norm]))

    def pv_tasks(h, steps):
        st = {}

        def pv(j):
            def fn():
                sl = slice(j * W // 8, (j + 1) * W // 8)
                part = jax.lax.dot_general(p_s[h & 1, :, sl].astype(bf16), kv_cols(v_b.at[h & 1], sl),
                                           (((1,), (1,)), ((), ())), preferred_element_type=f32)
                st["o"] = part if j == 0 else st["o"] + part
                if j == 7:
                    o_s[h] = st["o"]
            return fn

        return [(t, pv(j)) for j, t in enumerate(steps)]

    def q_tasks(i):
        def proj(t):
            def fn():
                cols = pl.ds(pl.multiple_of(128 * t, 128), 128)
                pr_s[t] = jnp.dot(x_rows(), wq_b[:, cols], preferred_element_type=f32)
            return fn

        return [(TW + 1 + 2 * j, proj(3 * i + j)) for j in range(3)]

    def gu_tasks(which):
        def proj(c):
            def fn():
                w = tile_column(gu_b.at[which], c, D // 8, F // 128)
                pr_s[(H * DH + F * which) // 128 + c] = jnp.dot(x_rows(), w, preferred_element_type=f32)
            return fn

        return [(2 * c, proj(c)) for c in range(F // 128)]

    def o_task(hd):
        def fn():
            w = jnp.concatenate([tile_column(wo_b, (NT_O // H) * hd + c, DH // 8, D // 128)
                                 for c in range(D // 128)], axis=1)
            a_s[...] += jnp.dot(o_s[hd].astype(bf16), w, preferred_element_type=f32)
        return fn

    def attn_tasks(i):
        return qk_tasks(i, TW + 8) + pv_tasks(i - 1, _every(LG, 8, 2))

    def stream_round(i, w_piece, tasks, first=False):
        by = _by_step(tasks)
        assert max(by) < NS
        for s in range(NS):
            if not first or s - LG >= -HS:
                kv_wait((s - LG) % NS)
            w_piece(i, s).start(priority=0)
            (kv_copy(0, i + 1, s, s) if s < HS else kv_copy(1, i, s - HS, s)).start(priority=1)
            if s == TW and first:
                tiles_wait(12 * RUN, p_sem.at[3])
                first_block = wq_b.at[:, pl.ds(0, QB)]
                pltpu.make_async_copy(first_block, first_block, p_sem.at[4]).wait()
                for c in small:
                    c.wait()
            elif s == TW:
                tiles_wait(4 * NS, w_sem.at[(i - 1) & 1])
            for fn in by.get(s, []):
                fn()

    def stream_rounds(lo, hi, w_piece, tasks):
        def body(i, carry):
            stream_round(i, w_piece, tasks(i) + attn_tasks(i))
            return carry
        jax.lax.fori_loop(lo, hi, body, 0)

    for j in range(D // 8 + HS):
        if j >= 16:
            run, part = divmod(j - 16, 8)
            run_piece((wg, wu)[run % 2], gu_b.at[run % 2], 0, 8 * (run // 2) + part, OFF_F,
                      p_sem.at[3]).start(priority=0)
        if j < D // 8:
            wq_copy(5 * (j % 16) + j // 16, 0, QB, p_sem.at[4]).start(priority=1)
        else:
            kv_copy(0, 0, j - D // 8, HS + j - D // 8).start(priority=1)
        if j == 60:
            for c in small:
                c.start()
    a_s[...] = jnp.zeros(a_s.shape, f32)

    def wo_piece(i, s, may_wrap=False):
        return run_piece(wo, wo_b, 4 * (i - 16), s, OFF_O, w_sem.at[i & 1], may_wrap)

    stream_round(0, wq_piece, q_tasks(0) + qk_tasks(0, TW + 8), first=True)
    stream_rounds(1, 10, wq_piece, q_tasks)
    stream_rounds(10, 13, lambda i, s: run_piece(wg, gu_b.at[0], 3 + 4 * (i - 10), s, OFF_F, w_sem.at[i & 1]), q_tasks)
    stream_rounds(13, 16, lambda i, s: run_piece(wu, gu_b.at[1], 3 + 4 * (i - 13), s, OFF_F, w_sem.at[i & 1]), q_tasks)
    stream_rounds(16, 18, lambda i, s: wo_piece(i, s, True), lambda i: gu_tasks(i - 16))
    stream_rounds(18, 30, wo_piece, lambda i: [(TW + 1, o_task(i - 18)), (TW + 4, o_task(i - 2))])

    st = {}

    def gates():
        xf = x_v[0].astype(f32)
        st["gate"] = jax.nn.sigmoid(jnp.sum(xf * gw_v[...].astype(f32).reshape(1, D), axis=-1, keepdims=True))
        st["rsel"] = jax.nn.sigmoid(jnp.sum(xf * wr_v[...].astype(f32).reshape(1, D), axis=-1, keepdims=True))

    def act():
        g, u = (jnp.concatenate([pr_s[(H * DH + F * which) // 128 + k] for k in range(F // 128)], axis=1)
                for which in range(2))
        st["h"] = jax.nn.silu(g) * u

    def h_column(j):
        def fn():
            hb_s[128 * j:128 * (j + 1)] = jnp.broadcast_to(st["h"][0:1, 128 * j:128 * (j + 1)], (128, 128)).T
        return fn

    y = {}

    def down(t0, n):
        for t in range(t0, t0 + n):
            r, c = divmod(t, D // 128)
            part = wd_b[t].astype(f32) * hb_s[8 * r:8 * r + 8]
            y[c] = y[c] + part if c in y else part

    stream_round(30, wo_piece,
                 [(0, gates), (2, act)] + [(3 + j, h_column(j)) for j in range(F // 128)]
                 + [(TW + 1, o_task(12)), (TW + 4, o_task(28))] + attn_tasks(30))

    landed = [LG + max(j for j, p in enumerate(ORDER[1]) if p[1] == c) for c in range(4)]
    t30 = [max(landed[j // 2] + HS - NS, 38 + 2 * j) for j in range(8)]
    t31 = [landed[j // 2] + 2 * (j % 2) for j in range(8)]
    assert landed == sorted(landed)
    by = _by_step([(2, o_task(13)), (6, o_task(29))] + qk_tasks(31, LG - HS)
                  + pv_tasks(30, t30) + [(t30[-1] + 3 * (j + 1), o_task(hd)) for j, hd in enumerate((30, 14, 15))]
                  + pv_tasks(31, t31) + [(t31[-1] + 2, o_task(31))])
    hi_pieces = [(RUN * ((k % 2) * (N_HI // 2) + k // 2) - OFF_F + u) % NT_F
                 for k in range(N_HI) for u in range(0, RUN, 4)]
    n_lo = NT_F // RUN - N_HI
    lo_pieces = [RUN * (N_HI + (k % 3) * (n_lo // 3) + k // 3) - OFF_F + u
                 for k in range(n_lo) for u in (0, RUN // 2)]
    n_steps = HS + len(lo_pieces) + LG
    assert len(hi_pieces) + TW < n_steps and max(by) + 1 < n_steps
    for s in range(n_steps):
        k, part = divmod(s - TW, 8)
        if part == 0 and 1 <= k <= N_HI:
            tiles_wait(RUN, d_sem.at[k - 1])
            for t in hi_pieces[8 * (k - 1):8 * k]:
                down(t, 4)
        if s == max(by) + 1:
            xf = x_v[0].astype(f32)
            y_scale = (1.0 - st["gate"]) * st["rsel"]
            rest = st["gate"] * a_s[0:1] + (1.0 - st["gate"]) * (xf + xf * 0.0)
        if s - LG < HS:
            kv_wait((s - LG) % NS)
        else:
            tiles_wait(RUN // 2, d_sem.at[N_HI + s - LG - HS])
            down(lo_pieces[s - LG - HS], RUN // 2)
        if s < len(hi_pieces):
            tiles_copy(wd, wd_b, hi_pieces[s], 4, d_sem.at[s // 8]).start(priority=0)
        if s < HS:
            kv_copy(1, H - 1, s, s).start(priority=1)
        elif s - HS < len(lo_pieces):
            tiles_copy(wd, wd_b, lo_pieces[s - HS], RUN // 2, d_sem.at[N_HI + s - HS]).start(priority=1)
        if s == TW:
            tiles_wait(4 * NS, w_sem.at[0])
        for fn in by.get(s, []):
            fn()

    y_row = jnp.sum(jnp.concatenate([y[c] for c in range(D // 128)], axis=1), axis=0, keepdims=True)
    out_ref[0] = (rest + y_scale * y_row).astype(bf16)


def _tiles(a):
    r, c = a.shape
    return a.reshape(r // 8, 8, c // 128, 128).transpose(0, 2, 1, 3).reshape(-1, 8, 128)


@jax.jit
def pallas_gated_mix__sliding_block_cached__moe_arch_mod__decode_kernel(
        A_x, A_k_cache, A_v_cache, A_wq, A_wo, B_x, B_w_r, B_w_gate, B_w_up, B_w_down, gate_w):
    del B_x
    kT = jnp.swapaxes(A_k_cache, 2, 3).reshape(H, DH // 32, 32, SK)
    vT = jnp.swapaxes(A_v_cache, 2, 3).reshape(H, DH // 32, 32, SK)
    vmem, dma = pltpu.VMEM, pltpu.SemaphoreType.DMA
    return pl.pallas_call(
        _kernel,
        out_shape=jax.ShapeDtypeStruct((1, 1, D), bf16),
        in_specs=[pl.BlockSpec(memory_space=pl.ANY)] * 10,
        out_specs=pl.BlockSpec(memory_space=pltpu.VMEM),
        scratch_shapes=[
            vmem((1, 1, D), bf16), vmem((D,), bf16), vmem((D,), bf16),
            vmem((2, DH // 32, 32, W), bf16), vmem((2, DH // 32, 32, W), bf16), vmem((D, H * DH), bf16),
            vmem((NT_O, 8, 128), bf16), vmem((2, NT_F, 8, 128), bf16), vmem((NT_F, 8, 128), bf16),
            vmem(((H * DH + 2 * F) // 128, M, 128), f32), vmem((H, M, DH), f32),
            vmem((M, W), f32), vmem((2, M, W), f32), vmem((M, D), f32), vmem((F, 128), f32),
            dma((NS,)), dma((2,)), dma((2 * NT_F // RUN - N_HI,)), dma((5,)),
        ],
        compiler_params=pltpu.CompilerParams(
            vmem_limit_bytes=64 * 1024 * 1024,
            disable_semaphore_checks=True,
            disable_bounds_checks=True,
        ),
        name="gated_mix_decode",
    )(A_x, kT, vT, A_wq, _tiles(A_wo), B_w_r, _tiles(B_w_gate), _tiles(B_w_up), _tiles(B_w_down), gate_w)
```

```python
import jax
import jax.numpy as jnp
import jax.experimental.pallas as pl
import jax.experimental.pallas.tpu as pltpu

H, DH, SK, D, F = 32, 192, 32768, 640, 1536
W = min(4096, max(256, SK // 4))
BASE = SK - W
M = 8

NS, HS = 64, 32
KC = W // 4
QB = 2048
RUN = 32
NT_O, NT_F = H * DH * D // 1024, F * D // 1024
OFF_O, OFF_F = 16, 8
N_HI = 12
LG = 46
TW = 15

f32, bf16 = jnp.float32, jnp.bfloat16


def _sweep(group, quarters):
    firsts = [0, 2, 12, 14, 1, 3, 13, 15]
    return [(r, c) for k in range(0, len(firsts), group) for c in quarters for r in firsts[k:k + group]]


ORDER = (_sweep(2, (0, 1)) + _sweep(2, (2, 3)),
         _sweep(4, (0, 1, 2)) + _sweep(4, (3,)))


def _complete(which, quarter):
    return max(j for j, p in enumerate(ORDER[which]) if p[1] == quarter)


def _every(t0, n, d):
    return [t0 + j * d for j in range(n)]


def _by_step(tasks):
    by = {}
    for t, fn in tasks:
        by.setdefault(t, []).append(fn)
    return by


def _kernel(x_hbm, kT, vT, wq, wo, wr_hbm, wg, wu, wd, gw_hbm, out_ref,
            x_v, wr_v, gw_v, k_b, v_b, wq_b, wo_b, gu_b, wd_b, pr_s, o_s, s_s, p_s, a_s, hb_s,
            kv_sem, w_sem, d_sem, p_sem):
    def kv_copy(which, h, j, slot):
        src, buf = (kT, vT)[which].at[h], (k_b, v_b)[which].at[h & 1]
        r, c = ORDER[which][j]
        groups, rows = pl.ds(r // 4, 3), pl.ds(8 * (r % 4), 8)
        return pltpu.make_async_copy(src.at[groups, rows, pl.ds(BASE + c * KC, KC)],
                                     buf.at[groups, rows, pl.ds(c * KC, KC)], kv_sem.at[slot])

    def kv_wait(slot):
        kv_copy(0, 0, 0, slot).wait()

    def tiles_copy(src, dst, t, n, sem):
        return pltpu.make_async_copy(src.at[pl.ds(t, n)], dst.at[pl.ds(t, n)], sem)

    def tiles_wait(n, sem):
        tiles_copy(wo_b, wo_b, 0, n, sem).wait()

    def wq_copy(row_tile, col, n, sem):
        idx = (pl.ds(pl.multiple_of(8 * row_tile, 8), 8), pl.ds(pl.multiple_of(col, 512), n))
        return pltpu.make_async_copy(wq.at[idx], wq_b.at[idx], sem)

    def wq_piece(i, s):
        blk = i // 5 if isinstance(i, int) else jnp.where(i >= 5, 1, 0)
        return wq_copy(5 * (s // 4) + i - 5 * blk, QB * (blk + 1) + 512 * (s % 4), 512, w_sem.at[i & 1])

    def run_piece(src, dst, pos, s, off, sem, may_wrap=False):
        n = src.shape[0]
        run, part = divmod(s, 8)
        t = (run % 2) * (n // 2) + (pos + run // 2) * RUN + 4 * part - off
        if isinstance(t, int):
            t %= n
        elif may_wrap and run == 0 and 4 * part < off:
            t = jnp.where(t < 0, t + n, t)
        return tiles_copy(src, dst, t, 4, sem)

    small = [pltpu.make_async_copy(x_hbm, x_v, p_sem.at[0]),
             pltpu.make_async_copy(gw_hbm, gw_v, p_sem.at[1]),
             pltpu.make_async_copy(wr_hbm, wr_v, p_sem.at[2])]

    def kv_cols(buf, sl):
        t = buf[:, :, sl]
        return t.reshape(DH, t.shape[-1])

    def tile_column(ref, t0, n, stride):
        return jnp.concatenate([ref[t0 + stride * k] for k in range(n)], axis=0)

    def x_rows():
        return jnp.broadcast_to(x_v[0], (M, D))

    def qk_tasks(h, t0):
        st = {}

        def qk(j):
            def fn():
                if j == 0:
                    tile = (3 * h) >> 1
                    q2 = jnp.concatenate([pr_s[tile], pr_s[tile + 1]], axis=1)
                    if isinstance(h, int):
                        q = q2[:, 64 * (h % 2):64 * (h % 2) + DH]
                    else:
                        q = jnp.where((h & 1) == 0, q2[:, :DH], q2[:, 64:])
                    st["q"] = q.astype(bf16)
                sl = slice(j * W // 8, (j + 1) * W // 8)
                s_s[:, sl] = jnp.dot(st["q"], kv_cols(k_b.at[h & 1], sl),
                                     preferred_element_type=f32) * (DH ** -0.5)
            return fn

        def sm_max():
            st["m"] = jnp.max(s_s[...], axis=-1, keepdims=True)

        def sm_exp():
            e = jnp.exp(s_s[...] - st["m"])
            s_s[...] = e
            st["l"] = jnp.sum(e, axis=-1, keepdims=True)

        def sm_norm():
            p_s[h & 1] = s_s[...] * (1.0 / st["l"])

        return list(zip(_every(t0, 11, 2), [qk(j) for j in range(8)] + [sm_max, sm_exp, sm_norm]))

    def pv_tasks(h, steps):
        st = {}

        def pv(j):
            def fn():
                sl = slice(j * W // 8, (j + 1) * W // 8)
                part = jax.lax.dot_general(p_s[h & 1, :, sl].astype(bf16), kv_cols(v_b.at[h & 1], sl),
                                           (((1,), (1,)), ((), ())), preferred_element_type=f32)
                st["o"] = part if j == 0 else st["o"] + part
                if j == 7:
                    o_s[h] = st["o"]
            return fn

        return [(t, pv(j)) for j, t in enumerate(steps)]

    def q_tasks(i):
        def proj(t):
            def fn():
                cols = pl.ds(pl.multiple_of(128 * t, 128), 128)
                pr_s[t] = jnp.dot(x_rows(), wq_b[:, cols], preferred_element_type=f32)
            return fn

        return [(TW + 1 + 2 * j, proj(3 * i + j)) for j in range(3)]

    def gu_tasks(which):
        def proj(c):
            def fn():
                w = tile_column(gu_b.at[which], c, D // 8, F // 128)
                pr_s[(H * DH + F * which) // 128 + c] = jnp.dot(x_rows(), w, preferred_element_type=f32)
            return fn

        return [(2 * c, proj(c)) for c in range(F // 128)]

    def o_task(hd):
        def fn():
            w = jnp.concatenate([tile_column(wo_b, (NT_O // H) * hd + c, DH // 8, D // 128)
                                 for c in range(D // 128)], axis=1)
            a_s[...] += jnp.dot(o_s[hd].astype(bf16), w, preferred_element_type=f32)
        return fn

    def attn_tasks(i):
        assert TW + 8 >= LG - HS
        return qk_tasks(i, TW + 8) + pv_tasks(i - 1, _every(LG, 8, 2))

    def stream_round(i, w_piece, tasks, first=False):
        by = _by_step(tasks)
        assert max(by) < NS
        for s in range(NS):
            if not first or s - LG >= -HS:
                kv_wait((s - LG) % NS)
            w_piece(i, s).start(priority=0)
            (kv_copy(0, i + 1, s, s) if s < HS else kv_copy(1, i, s - HS, s)).start(priority=1)
            if s == TW and first:
                tiles_wait(12 * RUN, p_sem.at[3])
                first_block = wq_b.at[:, pl.ds(0, QB)]
                pltpu.make_async_copy(first_block, first_block, p_sem.at[4]).wait()
                for c in small:
                    c.wait()
            elif s == TW:
                tiles_wait(4 * NS, w_sem.at[(i - 1) & 1])
            for fn in by.get(s, []):
                fn()

    def stream_rounds(lo, hi, w_piece, tasks):
        def body(i, carry):
            stream_round(i, w_piece, tasks(i) + attn_tasks(i))
            return carry
        jax.lax.fori_loop(lo, hi, body, 0)

    for j in range(D // 8 + HS):
        if j >= 16:
            run, part = divmod(j - 16, 8)
            run_piece((wg, wu)[run % 2], gu_b.at[run % 2], 0, 8 * (run // 2) + part, OFF_F,
                      p_sem.at[3]).start(priority=0)
        if j < D // 8:
            wq_copy(5 * (j % 16) + j // 16, 0, QB, p_sem.at[4]).start(priority=1)
        else:
            kv_copy(0, 0, j - D // 8, HS + j - D // 8).start(priority=1)
        if j == 60:
            for c in small:
                c.start()
    a_s[...] = jnp.zeros(a_s.shape, f32)

    def wo_piece(i, s, may_wrap=False):
        return run_piece(wo, wo_b, 4 * (i - 16), s, OFF_O, w_sem.at[i & 1], may_wrap)

    assert all(LG - HS + _complete(0, j // 2) <= 42 + 2 * j for j in range(8))
    stream_round(0, wq_piece, q_tasks(0) + qk_tasks(0, 42), first=True)
    stream_rounds(1, 10, wq_piece, q_tasks)
    stream_rounds(10, 13, lambda i, s: run_piece(wg, gu_b.at[0], 3 + 4 * (i - 10), s, OFF_F, w_sem.at[i & 1]), q_tasks)
    stream_rounds(13, 16, lambda i, s: run_piece(wu, gu_b.at[1], 3 + 4 * (i - 13), s, OFF_F, w_sem.at[i & 1]), q_tasks)
    stream_rounds(16, 18, lambda i, s: wo_piece(i, s, True), lambda i: gu_tasks(i - 16))
    stream_rounds(18, 30, wo_piece, lambda i: [(TW + 1, o_task(i - 18)), (TW + 4, o_task(i - 2))])

    st = {}

    def gates():
        xf = x_v[0].astype(f32)
        st["gate"] = jax.nn.sigmoid(jnp.sum(xf * gw_v[...].astype(f32).reshape(1, D), axis=-1, keepdims=True))
        st["rsel"] = jax.nn.sigmoid(jnp.sum(xf * wr_v[...].astype(f32).reshape(1, D), axis=-1, keepdims=True))

    def act():
        g, u = (jnp.concatenate([pr_s[(H * DH + F * which) // 128 + k] for k in range(F // 128)], axis=1)
                for which in range(2))
        st["h"] = jax.nn.silu(g) * u

    def h_column(j):
        def fn():
            hb_s[128 * j:128 * (j + 1)] = jnp.broadcast_to(st["h"][0:1, 128 * j:128 * (j + 1)], (128, 128)).T
        return fn

    y = {}

    def down(t0, n):
        for t in range(t0, t0 + n):
            r, c = divmod(t, D // 128)
            part = wd_b[t].astype(f32) * hb_s[8 * r:8 * r + 8]
            y[c] = y[c] + part if c in y else part

    stream_round(30, wo_piece,
                 [(0, gates), (2, act)] + [(3 + j, h_column(j)) for j in range(F // 128)]
                 + [(TW + 1, o_task(12)), (TW + 4, o_task(28))] + attn_tasks(30))

    landed = [LG + _complete(1, c) for c in range(4)]
    t30 = [max(landed[j // 2] + HS - NS, 38 + 2 * j) for j in range(8)]
    t31 = [landed[j // 2] + 2 * (j % 2) for j in range(8)]
    assert landed == sorted(landed)
    by = _by_step([(2, o_task(13)), (6, o_task(29))] + qk_tasks(31, LG - HS)
                  + pv_tasks(30, t30) + [(t30[-1] + 3 * (j + 1), o_task(hd)) for j, hd in enumerate((30, 14, 15))]
                  + pv_tasks(31, t31) + [(t31[-1] + 2, o_task(31))])
    hi_pieces = [(RUN * ((k % 2) * (N_HI // 2) + k // 2) - OFF_F + u) % NT_F
                 for k in range(N_HI) for u in range(0, RUN, 4)]
    n_lo = NT_F // RUN - N_HI
    lo_pieces = [RUN * (N_HI + (k % 3) * (n_lo // 3) + k // 3) - OFF_F + u
                 for k in range(n_lo) for u in (0, RUN // 2)]
    n_steps = HS + len(lo_pieces) + LG
    assert len(hi_pieces) + TW < n_steps and max(by) + 1 < n_steps
    for s in range(n_steps):
        k, part = divmod(s - TW, 8)
        if part == 0 and 1 <= k <= N_HI:
            tiles_wait(RUN, d_sem.at[k - 1])
            for t in hi_pieces[8 * (k - 1):8 * k]:
                down(t, 4)
        if s == max(by) + 1:
            xf = x_v[0].astype(f32)
            y_scale = (1.0 - st["gate"]) * st["rsel"]
            rest = st["gate"] * a_s[0:1] + (1.0 - st["gate"]) * (xf + xf * 0.0)
        if s - LG < HS:
            kv_wait((s - LG) % NS)
        else:
            tiles_wait(RUN // 2, d_sem.at[N_HI + s - LG - HS])
            down(lo_pieces[s - LG - HS], RUN // 2)
        if s < len(hi_pieces):
            tiles_copy(wd, wd_b, hi_pieces[s], 4, d_sem.at[s // 8]).start(priority=0)
        if s < HS:
            kv_copy(1, H - 1, s, s).start(priority=1)
        elif s - HS < len(lo_pieces):
            tiles_copy(wd, wd_b, lo_pieces[s - HS], RUN // 2, d_sem.at[N_HI + s - HS]).start(priority=1)
        if s == TW:
            tiles_wait(4 * NS, w_sem.at[0])
        for fn in by.get(s, []):
            fn()

    y_row = jnp.sum(jnp.concatenate([y[c] for c in range(D // 128)], axis=1), axis=0, keepdims=True)
    out_ref[0] = (rest + y_scale * y_row).astype(bf16)


def _tiles(a):
    r, c = a.shape
    return a.reshape(r // 8, 8, c // 128, 128).transpose(0, 2, 1, 3).reshape(-1, 8, 128)


@jax.jit
def pallas_gated_mix__sliding_block_cached__moe_arch_mod__decode_kernel(
        A_x, A_k_cache, A_v_cache, A_wq, A_wo, B_x, B_w_r, B_w_gate, B_w_up, B_w_down, gate_w):
    del B_x
    kT = jnp.swapaxes(A_k_cache, 2, 3).reshape(H, DH // 32, 32, SK)
    vT = jnp.swapaxes(A_v_cache, 2, 3).reshape(H, DH // 32, 32, SK)
    vmem, dma = pltpu.VMEM, pltpu.SemaphoreType.DMA
    return pl.pallas_call(
        _kernel,
        out_shape=jax.ShapeDtypeStruct((1, 1, D), bf16),
        in_specs=[pl.BlockSpec(memory_space=pl.ANY)] * 10,
        out_specs=pl.BlockSpec(memory_space=pltpu.VMEM),
        scratch_shapes=[
            vmem((1, 1, D), bf16), vmem((D,), bf16), vmem((D,), bf16),
            vmem((2, DH // 32, 32, W), bf16), vmem((2, DH // 32, 32, W), bf16), vmem((D, H * DH), bf16),
            vmem((NT_O, 8, 128), bf16), vmem((2, NT_F, 8, 128), bf16), vmem((NT_F, 8, 128), bf16),
            vmem(((H * DH + 2 * F) // 128, M, 128), f32), vmem((H, M, DH), f32),
            vmem((M, W), f32), vmem((2, M, W), f32), vmem((M, D), f32), vmem((F, 128), f32),
            dma((NS,)), dma((2,)), dma((2 * NT_F // RUN - N_HI,)), dma((5,)),
        ],
        compiler_params=pltpu.CompilerParams(
            vmem_limit_bytes=64 * 1024 * 1024,
            disable_semaphore_checks=True,
            disable_bounds_checks=True,
        ),
        name="gated_mix_decode",
    )(A_x, kT, vT, A_wq, _tiles(A_wo), B_w_r, _tiles(B_w_gate), _tiles(B_w_up), _tiles(B_w_down), gate_w)
```

```python
import jax
import jax.numpy as jnp
import jax.experimental.pallas as pl
import jax.experimental.pallas.tpu as pltpu

H, DH, SK, D, F = 32, 192, 32768, 640, 1536
W = min(4096, max(256, SK // 4))
BASE = SK - W
M = 8

NS, HS = 64, 32
KC = W // 4
QB = 2048
RUN = 32
NT_O, NT_F = H * DH * D // 1024, F * D // 1024
OFF_O, OFF_F = 16, 8
N_HI = 12
LG = 46
TW, TE = 16, 20
T_GATE, T_UP = H * DH // 128, (H * DH + F) // 128

f32, bf16 = jnp.float32, jnp.bfloat16


def _sweep(group, quarters):
    firsts = [0, 2, 12, 14, 1, 3, 13, 15]
    return [(r, c) for k in range(0, len(firsts), group) for c in quarters for r in firsts[k:k + group]]


ORDER = (_sweep(2, (0, 1)) + _sweep(2, (2, 3)),
         _sweep(4, (0, 1, 2)) + _sweep(4, (3,)))


def _complete(which, quarter):
    return max(j for j, p in enumerate(ORDER[which]) if p[1] == quarter)


def _every(t0, n, d):
    return [t0 + j * d for j in range(n)]


def _by_step(tasks):
    by = {}
    for t, fn in tasks:
        by.setdefault(t, []).append(fn)
    return by


def _kernel(x_hbm, kT, vT, wq, wo, wr_hbm, wg, wu, wd, gw_hbm, out_ref,
            x_v, wr_v, gw_v, k_b, v_b, wq_b, wo_b, gu_b, wd_b, pr_s, o_s, s_s, p_s, a_s, g_s, hb_s,
            kv_sem, w_sem, d_sem, p_sem):
    def kv_copy(which, h, j, slot):
        src, buf = (kT, vT)[which].at[h], (k_b, v_b)[which].at[h & 1]
        r, c = ORDER[which][j]
        groups, rows = pl.ds(r // 4, 3), pl.ds(8 * (r % 4), 8)
        return pltpu.make_async_copy(src.at[groups, rows, pl.ds(BASE + c * KC, KC)],
                                     buf.at[groups, rows, pl.ds(c * KC, KC)], kv_sem.at[slot])

    def kv_wait(slot):
        kv_copy(0, 0, 0, slot).wait()

    def tiles_copy(src, dst, t, n, sem):
        return pltpu.make_async_copy(src.at[pl.ds(t, n)], dst.at[pl.ds(t, n)], sem)

    def tiles_wait(n, sem):
        tiles_copy(wo_b, wo_b, 0, n, sem).wait()

    def wq_copy(row_tile, col, n, sem):
        idx = (pl.ds(pl.multiple_of(8 * row_tile, 8), 8), pl.ds(pl.multiple_of(col, 512), n))
        return pltpu.make_async_copy(wq.at[idx], wq_b.at[idx], sem)

    def wq_piece(i, s):
        blk = i // 5 if isinstance(i, int) else jnp.where(i >= 5, 1, 0)
        return wq_copy(5 * (s // 4) + i - 5 * blk, QB * (blk + 1) + 512 * (s % 4), 512, w_sem.at[i & 1])

    def run_piece(src, dst, pos, s, off, sem, may_wrap=False):
        n = src.shape[0]
        run, part = divmod(s, 8)
        t = (run % 2) * (n // 2) + (pos + run // 2) * RUN + 4 * part - off
        if isinstance(t, int):
            t %= n
        elif may_wrap and run == 0 and 4 * part < off:
            t = jnp.where(t < 0, t + n, t)
        return tiles_copy(src, dst, t, 4, sem)

    small = [pltpu.make_async_copy(x_hbm, x_v, p_sem.at[0]),
             pltpu.make_async_copy(gw_hbm, gw_v, p_sem.at[1]),
             pltpu.make_async_copy(wr_hbm, wr_v, p_sem.at[2])]

    def kv_cols(buf, sl):
        t = buf[:, :, sl]
        return t.reshape(DH, t.shape[-1])

    def tile_column(ref, t0, n, stride):
        return jnp.concatenate([ref[t0 + stride * k] for k in range(n)], axis=0)

    def x_rows():
        return jnp.broadcast_to(x_v[0], (M, D))

    def qk_tasks(h, t0):
        st = {}

        def qk(j):
            def fn():
                if j == 0:
                    tile = (3 * h) >> 1
                    q2 = jnp.concatenate([pr_s[tile], pr_s[tile + 1]], axis=1)
                    if isinstance(h, int):
                        q = q2[:, 64 * (h % 2):64 * (h % 2) + DH]
                    else:
                        q = jnp.where((h & 1) == 0, q2[:, :DH], q2[:, 64:])
                    st["q"] = q.astype(bf16)
                sl = slice(j * W // 8, (j + 1) * W // 8)
                s_s[:, sl] = jnp.dot(st["q"], kv_cols(k_b.at[h & 1], sl),
                                     preferred_element_type=f32) * (DH ** -0.5)
            return fn

        def sm_max():
            st["m"] = jnp.max(s_s[...], axis=-1, keepdims=True)

        def sm_exp():
            e = jnp.exp(s_s[...] - st["m"])
            s_s[...] = e
            st["l"] = jnp.sum(e, axis=-1, keepdims=True)

        def sm_norm():
            p_s[h & 1] = s_s[...] * (1.0 / st["l"])

        return list(zip(_every(t0, 11, 2), [qk(j) for j in range(8)] + [sm_max, sm_exp, sm_norm]))

    def pv_tasks(h, steps):
        st = {}

        def pv(j):
            def fn():
                sl = slice(j * W // 8, (j + 1) * W // 8)
                part = jax.lax.dot_general(p_s[h & 1, :, sl].astype(bf16), kv_cols(v_b.at[h & 1], sl),
                                           (((1,), (1,)), ((), ())), preferred_element_type=f32)
                st["o"] = part if j == 0 else st["o"] + part
                if j == 7:
                    o_s[h] = st["o"]
            return fn

        return [(t, pv(j)) for j, t in enumerate(steps)]

    def q_tasks(i):
        def proj(t):
            def fn():
                cols = pl.ds(pl.multiple_of(128 * t, 128), 128)
                pr_s[t] = jnp.dot(x_rows(), wq_b[:, cols], preferred_element_type=f32)
            return fn

        return [(TW + 1 + 2 * j, proj(3 * i + j)) for j in range(3)]

    def gu_tasks(which):
        def proj(c):
            def fn():
                w = jnp.concatenate([tile_column(gu_b.at[which], c + u, D // 8, F // 128) for u in range(2)], axis=1)
                v = jnp.dot(x_rows(), w, preferred_element_type=f32)
                for u in range(2):
                    pr_s[T_GATE + (T_UP - T_GATE) * which + c + u] = v[:, 128 * u:128 * (u + 1)]
            return fn

        return [(2 * c, proj(c)) for c in range(0, F // 128, 2)]

    def gates():
        xf = x_rows().astype(f32)
        for k, w in enumerate((gw_v, wr_v)):
            logit = jnp.sum(xf * w[...].astype(f32).reshape(1, D), axis=-1, keepdims=True)
            g_s[k] = jnp.broadcast_to(jax.nn.sigmoid(logit), (M, 128))

    def h_task(j):
        def fn():
            h = jax.nn.silu(pr_s[T_GATE + j]) * pr_s[T_UP + j] * ((1.0 - g_s[0]) * g_s[1])
            hb_s[j] = jnp.concatenate([h] * (128 // M), axis=0).T
        return fn

    def o_task(hd):
        def fn():
            w = jnp.concatenate([tile_column(wo_b, (NT_O // H) * hd + c, DH // 8, D // 128)
                                 for c in range(D // 128)], axis=1)
            a_s[...] += jnp.dot(o_s[hd].astype(bf16), w, preferred_element_type=f32)
        return fn

    def attn_tasks(i):
        assert TW + 8 >= LG - HS
        return qk_tasks(i, TW + 8) + pv_tasks(i - 1, _every(LG + 2, 8, 2))

    def stream_round(i, w_piece, tasks, first=False):
        by = _by_step(tasks)
        assert max(by) < NS
        for s in range(NS):
            if not first or s - LG >= -HS:
                kv_wait((s - LG) % NS)
            (kv_copy(0, i + 1, s, s) if s < HS else kv_copy(1, i, s - HS, s)).start(priority=1)
            w_piece(i, s).start(priority=0)
            if s == TW and first:
                tiles_wait(12 * RUN, p_sem.at[3])
                first_block = wq_b.at[:, pl.ds(0, QB)]
                pltpu.make_async_copy(first_block, first_block, p_sem.at[4]).wait()
                for c in small:
                    c.wait()
            elif s == TW:
                tiles_wait(4 * NS, w_sem.at[(i - 1) & 1])
            for fn in by.get(s, []):
                fn()

    def stream_rounds(lo, hi, w_piece, tasks):
        def body(i, carry):
            stream_round(i, w_piece, tasks(i) + attn_tasks(i))
            return carry
        jax.lax.fori_loop(lo, hi, body, 0)

    for j in range(D // 8 + HS):
        if j >= 16:
            run, part = divmod(j - 16, 8)
            run_piece((wg, wu)[run % 2], gu_b.at[run % 2], 0, 8 * (run // 2) + part, OFF_F,
                      p_sem.at[3]).start(priority=0)
        if j < D // 8:
            wq_copy(5 * (j % 16) + j // 16, 0, QB, p_sem.at[4]).start(priority=1)
        else:
            kv_copy(0, 0, j - D // 8, HS + j - D // 8).start(priority=1)
        if j == 60:
            for c in small:
                c.start()
    a_s[...] = jnp.zeros(a_s.shape, f32)

    def wo_piece(i, s, may_wrap=False):
        return run_piece(wo, wo_b, 4 * (i - 16), s, OFF_O, w_sem.at[i & 1], may_wrap)

    assert all(LG - HS + _complete(0, j // 2) <= 42 + 2 * j for j in range(8))
    stream_round(0, wq_piece, q_tasks(0) + [(TW + 10, gates)] + qk_tasks(0, 42), first=True)
    stream_rounds(1, 10, wq_piece, q_tasks)
    stream_rounds(10, 13, lambda i, s: run_piece(wg, gu_b.at[0], 3 + 4 * (i - 10), s, OFF_F, w_sem.at[i & 1]), q_tasks)
    stream_rounds(13, 16, lambda i, s: run_piece(wu, gu_b.at[1], 3 + 4 * (i - 13), s, OFF_F, w_sem.at[i & 1]), q_tasks)
    stream_rounds(16, 18, lambda i, s: wo_piece(i, s, True), lambda i: gu_tasks(i - 16))
    stream_rounds(18, 31, wo_piece, lambda i: [(4, h_task(jnp.minimum(i - 18, F // 128 - 1))),
                                               (TW + 1, o_task(i - 2)), (TW + 4, o_task(i - 18))])

    y = {}

    def down(t0, n):
        for t in range(t0, t0 + n):
            r, c = divmod(t, D // 128)
            part = wd_b[t].astype(f32) * hb_s[r // 16, 8 * (r % 16):8 * (r % 16) + 8]
            y[c] = y[c] + part if c in y else part

    def mix():
        xf = x_rows().astype(f32)
        gate = jnp.concatenate([g_s[0]] * (D // 128), axis=1)
        rest = gate * a_s[...] + (1.0 - gate) * (xf + xf * 0.0)
        one_row = jax.lax.broadcasted_iota(jnp.int32, (M, 128), 0) == 0
        for c in range(D // 128):
            y[c] = y[c] + jnp.where(one_row, rest[:, 128 * c:128 * (c + 1)], 0.0)

    landed = [LG + _complete(1, c) for c in range(4)]
    t30 = [max(landed[j // 2] + HS - NS, 38 + 2 * j) for j in range(8)]
    t31 = [landed[j // 2] + 2 * (j % 2) for j in range(8)]
    assert landed == sorted(landed)
    by = _by_step([(2, o_task(13)), (6, o_task(29))] + qk_tasks(31, LG - HS)
                  + pv_tasks(30, t30) + [(t30[-1] + 3 * (j + 1), o_task(hd)) for j, hd in enumerate((30, 14, 15))]
                  + pv_tasks(31, t31) + [(t31[-1] + 2, o_task(31)), (t31[-1] + 3, mix)])
    hi_pieces = [(RUN * ((k % 2) * (N_HI // 2) + k // 2) - OFF_F + u) % NT_F
                 for k in range(N_HI) for u in range(0, RUN, 4)]
    n_lo = NT_F // RUN - N_HI
    lo_pieces = [RUN * (N_HI + (k % 2) * (n_lo // 2) + k // 2) - OFF_F + u
                 for k in range(n_lo) for u in (0, RUN // 2)]
    n_steps = HS + len(lo_pieces) + LG
    assert len(hi_pieces) < n_steps - 1 and max(by) < n_steps
    for s in range(n_steps):
        for k in range(N_HI):
            if s == min(8 * (k + 1) + TE + 1, n_steps - 1):
                tiles_wait(RUN, d_sem.at[k])
                for t in hi_pieces[8 * k:8 * (k + 1)]:
                    down(t, 4)
        if s - LG < HS:
            kv_wait((s - LG) % NS)
        else:
            tiles_wait(RUN // 2, d_sem.at[N_HI + s - LG - HS])
            down(lo_pieces[s - LG - HS], RUN // 2)
        if s < len(hi_pieces):
            tiles_copy(wd, wd_b, hi_pieces[s], 4, d_sem.at[s // 8]).start(priority=0)
        if s < HS:
            kv_copy(1, H - 1, s, s).start(priority=1)
        elif s - HS < len(lo_pieces):
            tiles_copy(wd, wd_b, lo_pieces[s - HS], RUN // 2, d_sem.at[N_HI + s - HS]).start(priority=1)
        if s == TW:
            tiles_wait(4 * NS, w_sem.at[0])
        for fn in by.get(s, []):
            fn()

    out = jnp.sum(jnp.concatenate([y[c] for c in range(D // 128)], axis=1), axis=0, keepdims=True)
    out_ref[0] = out.astype(bf16)


def _tiles(a):
    r, c = a.shape
    return a.reshape(r // 8, 8, c // 128, 128).transpose(0, 2, 1, 3).reshape(-1, 8, 128)


@jax.jit
def pallas_gated_mix__sliding_block_cached__moe_arch_mod__decode_kernel(
        A_x, A_k_cache, A_v_cache, A_wq, A_wo, B_x, B_w_r, B_w_gate, B_w_up, B_w_down, gate_w):
    del B_x
    kT = jnp.swapaxes(A_k_cache, 2, 3).reshape(H, DH // 32, 32, SK)
    vT = jnp.swapaxes(A_v_cache, 2, 3).reshape(H, DH // 32, 32, SK)
    vmem, dma = pltpu.VMEM, pltpu.SemaphoreType.DMA
    return pl.pallas_call(
        _kernel,
        out_shape=jax.ShapeDtypeStruct((1, 1, D), bf16),
        in_specs=[pl.BlockSpec(memory_space=pl.ANY)] * 10,
        out_specs=pl.BlockSpec(memory_space=pltpu.VMEM),
        scratch_shapes=[
            vmem((1, 1, D), bf16), vmem((D,), bf16), vmem((D,), bf16),
            vmem((2, DH // 32, 32, W), bf16), vmem((2, DH // 32, 32, W), bf16), vmem((D, H * DH), bf16),
            vmem((NT_O, 8, 128), bf16), vmem((2, NT_F, 8, 128), bf16), vmem((NT_F, 8, 128), bf16),
            vmem(((H * DH + 2 * F) // 128, M, 128), f32), vmem((H, M, DH), f32),
            vmem((M, W), f32), vmem((2, M, W), f32), vmem((M, D), f32),
            vmem((2, M, 128), f32), vmem((F // 128, 128, 128), f32),
            dma((NS,)), dma((2,)), dma((2 * NT_F // RUN - N_HI,)), dma((5,)),
        ],
        compiler_params=pltpu.CompilerParams(
            vmem_limit_bytes=64 * 1024 * 1024,
            disable_semaphore_checks=True,
            disable_bounds_checks=True,
        ),
        name="gated_mix_decode",
    )(A_x, kT, vT, A_wq, _tiles(A_wo), B_w_r, _tiles(B_w_gate), _tiles(B_w_up), _tiles(B_w_down), gate_w)
```

```python
import jax
import jax.numpy as jnp
import jax.experimental.pallas as pl
import jax.experimental.pallas.tpu as pltpu

H, DH, SK, D, F = 32, 192, 32768, 640, 1536
W = min(4096, max(256, SK // 4))
BASE = SK - W
M = 8

NS, HS = 64, 32
KC = W // 4
QB = 2048
RUN = 32
NT_O, NT_F = H * DH * D // 1024, F * D // 1024
OFF_O, OFF_F = 16, 8
N_HI = 12
LG = 46
TW, TE = 16, 20
T_GATE, T_UP = H * DH // 128, (H * DH + F) // 128

f32, bf16 = jnp.float32, jnp.bfloat16


def _sweep(group, quarters):
    firsts = [0, 2, 12, 14, 1, 3, 13, 15]
    return [(r, c) for k in range(0, len(firsts), group) for c in quarters for r in firsts[k:k + group]]


ORDER = (_sweep(2, (0, 1)) + _sweep(2, (2, 3)),
         _sweep(4, (0, 1, 2)) + _sweep(4, (3,)))


def _complete(which, quarter):
    return max(j for j, p in enumerate(ORDER[which]) if p[1] == quarter)


def _every(t0, n, d):
    return [t0 + j * d for j in range(n)]


def _by_step(tasks):
    by = {}
    for t, fn in tasks:
        by.setdefault(t, []).append(fn)
    return by


def _kernel(x_hbm, kT, vT, wq, wo, wr_hbm, wg, wu, wd, gw_hbm, out_ref,
            x_v, wr_v, gw_v, k_b, v_b, wq_b, wo_b, gu_b, wd_b, pr_s, o_s, s_s, p_s, a_s, g_s, hb_s,
            kv_sem, w_sem, d_sem, p_sem):
    def kv_copy(which, h, j, slot):
        src, buf = (kT, vT)[which].at[h], (k_b, v_b)[which].at[h & 1]
        r, c = ORDER[which][j]
        groups, rows = pl.ds(r // 4, 3), pl.ds(8 * (r % 4), 8)
        return pltpu.make_async_copy(src.at[groups, rows, pl.ds(BASE + c * KC, KC)],
                                     buf.at[groups, rows, pl.ds(c * KC, KC)], kv_sem.at[slot])

    def round_copy(i, s):
        return kv_copy(0, i + 1, s, s) if s < HS else kv_copy(1, i, s - HS, s)

    def tiles_copy(src, dst, t, n, sem):
        return pltpu.make_async_copy(src.at[pl.ds(t, n)], dst.at[pl.ds(t, n)], sem)

    def tiles_wait(n, sem):
        tiles_copy(wd_b, wd_b, 0, n, sem).wait()

    def wq_copy(row_tile, col, n, sem):
        idx = (pl.ds(pl.multiple_of(8 * row_tile, 8), 8), pl.ds(pl.multiple_of(col, 512), n))
        return pltpu.make_async_copy(wq.at[idx], wq_b.at[idx], sem)

    def wq_piece(i, s):
        blk = i // 5 if isinstance(i, int) else jnp.where(i >= 5, 1, 0)
        return wq_copy(5 * (s // 4) + i - 5 * blk, QB * (blk + 1) + 512 * (s % 4), 512, w_sem.at[i & 1])

    def run_piece(src, dst, pos, s, off, sem, may_wrap=False):
        n = src.shape[0]
        run, part = divmod(s, 8)
        t = (run % 2) * (n // 2) + (pos + run // 2) * RUN + 4 * part - off
        if isinstance(t, int):
            t %= n
        elif may_wrap and run == 0 and 4 * part < off:
            t = jnp.where(t < 0, t + n, t)
        return tiles_copy(src, dst, t, 4, sem)

    small = [pltpu.make_async_copy(x_hbm, x_v, p_sem.at[0]),
             pltpu.make_async_copy(gw_hbm, gw_v, p_sem.at[1]),
             pltpu.make_async_copy(wr_hbm, wr_v, p_sem.at[2])]

    def kv_cols(buf, sl):
        t = buf[:, :, sl]
        return t.reshape(DH, t.shape[-1])

    def tile_column(ref, t0, n, stride):
        return jnp.concatenate([ref[t0 + stride * k] for k in range(n)], axis=0)

    def x_rows():
        return jnp.broadcast_to(x_v[0], (M, D))

    def qk_tasks(h, t0):
        st = {}

        def qk(j):
            def fn():
                if j == 0:
                    tile = (3 * h) >> 1
                    q2 = jnp.concatenate([pr_s[tile], pr_s[tile + 1]], axis=1)
                    if isinstance(h, int):
                        q = q2[:, 64 * (h % 2):64 * (h % 2) + DH]
                    else:
                        q = jnp.where((h & 1) == 0, q2[:, :DH], q2[:, 64:])
                    st["q"] = q.astype(bf16)
                sl = slice(j * W // 8, (j + 1) * W // 8)
                s_s[:, sl] = jnp.dot(st["q"], kv_cols(k_b.at[h & 1], sl),
                                     preferred_element_type=f32) * (DH ** -0.5)
            return fn

        def sm_max():
            st["m"] = jnp.max(s_s[...], axis=-1, keepdims=True)

        def sm_exp():
            e = jnp.exp(s_s[...] - st["m"])
            s_s[...] = e
            st["l"] = jnp.sum(e, axis=-1, keepdims=True)

        def sm_norm():
            p_s[h & 1] = s_s[...] * (1.0 / st["l"])

        return list(zip(_every(t0, 11, 2), [qk(j) for j in range(8)] + [sm_max, sm_exp, sm_norm]))

    def pv_tasks(h, steps):
        st = {}

        def pv(j):
            def fn():
                sl = slice(j * W // 8, (j + 1) * W // 8)
                part = jax.lax.dot_general(p_s[h & 1, :, sl].astype(bf16), kv_cols(v_b.at[h & 1], sl),
                                           (((1,), (1,)), ((), ())), preferred_element_type=f32)
                st["o"] = part if j == 0 else st["o"] + part
                if j == 7:
                    o_s[h] = st["o"]
            return fn

        return [(t, pv(j)) for j, t in enumerate(steps)]

    def q_tasks(i):
        def proj(t):
            def fn():
                cols = pl.ds(pl.multiple_of(128 * t, 128), 128)
                pr_s[t] = jnp.dot(x_rows(), wq_b[:, cols], preferred_element_type=f32)
            return fn

        return [(TW + 1 + 2 * j, proj(3 * i + j)) for j in range(3)]

    def gu_tasks(which):
        def proj(c):
            def fn():
                w = jnp.concatenate([tile_column(gu_b.at[which], c + u, D // 8, F // 128) for u in range(2)], axis=1)
                v = jnp.dot(x_rows(), w, preferred_element_type=f32)
                for u in range(2):
                    pr_s[T_GATE + (T_UP - T_GATE) * which + c + u] = v[:, 128 * u:128 * (u + 1)]
            return fn

        return [(2 * c, proj(c)) for c in range(0, F // 128, 2)]

    def gates():
        xf = x_rows().astype(f32)
        for k, w in enumerate((gw_v, wr_v)):
            logit = jnp.sum(xf * w[...].astype(f32).reshape(1, D), axis=-1, keepdims=True)
            g_s[k] = jnp.broadcast_to(jax.nn.sigmoid(logit), (M, 128))

    def h_task(j):
        def fn():
            h = jax.nn.silu(pr_s[T_GATE + j]) * pr_s[T_UP + j] * ((1.0 - g_s[0]) * g_s[1])
            hb_s[j] = jnp.concatenate([h] * (128 // M), axis=0).T
        return fn

    def o_task(hd):
        def fn():
            w = jnp.concatenate([tile_column(wo_b, (NT_O // H) * hd + c, DH // 8, D // 128)
                                 for c in range(D // 128)], axis=1)
            a_s[...] += jnp.dot(o_s[hd].astype(bf16), w, preferred_element_type=f32)
        return fn

    def attn_tasks(i):
        assert TW + 8 >= LG - HS
        return qk_tasks(i, TW + 8) + pv_tasks(i - 1, _every(LG + 2, 8, 2))

    def stream_round(i, w_piece, tasks, first=False):
        by = _by_step(tasks)
        assert max(by) < NS
        for s in range(NS):
            if s >= LG:
                round_copy(i, s - LG).wait()
            elif not first:
                round_copy(i - 1, s - LG + NS).wait()
            elif s - LG >= -HS:
                kv_copy(0, 0, s - LG + HS, s - LG + NS).wait()
            round_copy(i, s).start(priority=1)
            w_piece(i, s).start(priority=0)
            if s == TW and first:
                tiles_wait(12 * RUN, p_sem.at[3])
                first_block = wq_b.at[:, pl.ds(0, QB)]
                pltpu.make_async_copy(first_block, first_block, p_sem.at[4]).wait()
                for c in small:
                    c.wait()
            elif s == TW:
                tiles_wait(4 * NS, w_sem.at[(i - 1) & 1])
            for fn in by.get(s, []):
                fn()

    def stream_rounds(lo, hi, w_piece, tasks):
        def body(i, carry):
            stream_round(i, w_piece, tasks(i) + attn_tasks(i))
            return carry
        jax.lax.fori_loop(lo, hi, body, 0)

    for j in range(D // 8 + HS):
        if j >= 16:
            run, part = divmod(j - 16, 8)
            run_piece((wg, wu)[run % 2], gu_b.at[run % 2], 0, 8 * (run // 2) + part, OFF_F,
                      p_sem.at[3]).start(priority=0)
        if j < D // 8:
            wq_copy(5 * (j % 16) + j // 16, 0, QB, p_sem.at[4]).start(priority=1)
        else:
            kv_copy(0, 0, j - D // 8, HS + j - D // 8).start(priority=1)
        if j == 60:
            for c in small:
                c.start()
    a_s[...] = jnp.zeros(a_s.shape, f32)

    def wo_piece(i, s, may_wrap=False):
        return run_piece(wo, wo_b, 4 * (i - 16), s, OFF_O, w_sem.at[i & 1], may_wrap)

    assert all(LG - HS + _complete(0, j // 2) <= 42 + 2 * j for j in range(8))
    stream_round(0, wq_piece, q_tasks(0) + [(TW + 10, gates)] + qk_tasks(0, 42), first=True)
    stream_rounds(1, 10, wq_piece, q_tasks)
    stream_rounds(10, 13, lambda i, s: run_piece(wg, gu_b.at[0], 3 + 4 * (i - 10), s, OFF_F, w_sem.at[i & 1]), q_tasks)
    stream_rounds(13, 16, lambda i, s: run_piece(wu, gu_b.at[1], 3 + 4 * (i - 13), s, OFF_F, w_sem.at[i & 1]), q_tasks)
    stream_rounds(16, 18, lambda i, s: wo_piece(i, s, True), lambda i: gu_tasks(i - 16))
    stream_rounds(18, 31, wo_piece, lambda i: [(4, h_task(jnp.minimum(i - 18, F // 128 - 1))),
                                               (TW + 1, o_task(i - 2)), (TW + 4, o_task(i - 18))])

    y = {}

    def down(t0, n):
        for t in range(t0, t0 + n):
            r, c = divmod(t, D // 128)
            part = wd_b[t].astype(f32) * hb_s[r // 16, 8 * (r % 16):8 * (r % 16) + 8]
            y[c] = y[c] + part if c in y else part

    def mix():
        xf = x_rows().astype(f32)
        gate = jnp.concatenate([g_s[0]] * (D // 128), axis=1)
        rest = gate * a_s[...] + (1.0 - gate) * (xf + xf * 0.0)
        one_row = jax.lax.broadcasted_iota(jnp.int32, (M, 128), 0) == 0
        for c in range(D // 128):
            y[c] = y[c] + jnp.where(one_row, rest[:, 128 * c:128 * (c + 1)], 0.0)

    landed = [LG + _complete(1, c) for c in range(4)]
    t30 = [max(landed[j // 2] + HS - NS, 38 + 2 * j) for j in range(8)]
    t31 = [landed[j // 2] + 2 * (j % 2) for j in range(8)]
    assert landed == sorted(landed)
    by = _by_step([(2, o_task(13)), (6, o_task(29))] + qk_tasks(31, LG - HS)
                  + pv_tasks(30, t30) + [(t30[-1] + 3 * (j + 1), o_task(hd)) for j, hd in enumerate((30, 14, 15))]
                  + pv_tasks(31, t31) + [(t31[-1] + 2, o_task(31)), (t31[-1] + 3, mix)])
    hi_pieces = [(RUN * ((k % 2) * (N_HI // 2) + k // 2) - OFF_F + u) % NT_F
                 for k in range(N_HI) for u in range(0, RUN, 4)]
    n_lo = NT_F // RUN - N_HI
    lo_pieces = [RUN * (N_HI + (k % 2) * (n_lo // 2) + k // 2) - OFF_F + u
                 for k in range(n_lo) for u in (0, RUN // 2)]
    n_steps = HS + len(lo_pieces) + LG
    assert len(hi_pieces) < n_steps - 1 and max(by) < n_steps
    for s in range(n_steps):
        for k in range(N_HI):
            if s == min(8 * (k + 1) + TE + 1, n_steps - 1):
                tiles_wait(RUN, d_sem.at[k])
                for t in hi_pieces[8 * k:8 * (k + 1)]:
                    down(t, 4)
        if s < LG:
            round_copy(H - 2, s - LG + NS).wait()
        elif s - LG < HS:
            kv_copy(1, H - 1, s - LG, s - LG).wait()
        else:
            tiles_copy(wd, wd_b, lo_pieces[s - LG - HS], RUN // 2, d_sem.at[N_HI + s - LG - HS]).wait()
            down(lo_pieces[s - LG - HS], RUN // 2)
        if s < len(hi_pieces):
            tiles_copy(wd, wd_b, hi_pieces[s], 4, d_sem.at[s // 8]).start(priority=0)
        if s < HS:
            kv_copy(1, H - 1, s, s).start(priority=1)
        elif s - HS < len(lo_pieces):
            tiles_copy(wd, wd_b, lo_pieces[s - HS], RUN // 2, d_sem.at[N_HI + s - HS]).start(priority=1)
        if s == TW:
            tiles_wait(4 * NS, w_sem.at[0])
        for fn in by.get(s, []):
            fn()

    out = jnp.sum(jnp.concatenate([y[c] for c in range(D // 128)], axis=1), axis=0, keepdims=True)
    out_ref[0] = out.astype(bf16)


def _tiles(a):
    r, c = a.shape
    return a.reshape(r // 8, 8, c // 128, 128).transpose(0, 2, 1, 3).reshape(-1, 8, 128)


@jax.jit
def pallas_gated_mix__sliding_block_cached__moe_arch_mod__decode_kernel(
        A_x, A_k_cache, A_v_cache, A_wq, A_wo, B_x, B_w_r, B_w_gate, B_w_up, B_w_down, gate_w):
    del B_x
    kT = jnp.swapaxes(A_k_cache, 2, 3).reshape(H, DH // 32, 32, SK)
    vT = jnp.swapaxes(A_v_cache, 2, 3).reshape(H, DH // 32, 32, SK)
    vmem, dma = pltpu.VMEM, pltpu.SemaphoreType.DMA
    return pl.pallas_call(
        _kernel,
        out_shape=jax.ShapeDtypeStruct((1, 1, D), bf16),
        in_specs=[pl.BlockSpec(memory_space=pl.ANY)] * 10,
        out_specs=pl.BlockSpec(memory_space=pltpu.VMEM),
        scratch_shapes=[
            vmem((1, 1, D), bf16), vmem((D,), bf16), vmem((D,), bf16),
            vmem((2, DH // 32, 32, W), bf16), vmem((2, DH // 32, 32, W), bf16), vmem((D, H * DH), bf16),
            vmem((NT_O, 8, 128), bf16), vmem((2, NT_F, 8, 128), bf16), vmem((NT_F, 8, 128), bf16),
            vmem(((H * DH + 2 * F) // 128, M, 128), f32), vmem((H, M, DH), f32),
            vmem((M, W), f32), vmem((2, M, W), f32), vmem((M, D), f32),
            vmem((2, M, 128), f32), vmem((F // 128, 128, 128), f32),
            dma((NS,)), dma((2,)), dma((2 * NT_F // RUN - N_HI,)), dma((5,)),
        ],
        compiler_params=pltpu.CompilerParams(
            vmem_limit_bytes=64 * 1024 * 1024,
            disable_semaphore_checks=True,
            disable_bounds_checks=True,
        ),
        name="gated_mix_decode",
    )(A_x, kT, vT, A_wq, _tiles(A_wo), B_w_r, _tiles(B_w_gate), _tiles(B_w_up), _tiles(B_w_down), gate_w)
```

```python
import jax
import jax.numpy as jnp
import jax.experimental.pallas as pl
import jax.experimental.pallas.tpu as pltpu

H, DH, SK, D, F = 32, 192, 32768, 640, 1536
W = min(4096, max(256, SK // 4))
BASE = SK - W
M = 8

NS, HS = 64, 32
RT = DH // 8
SHIFT = (5, 6)
KC = W // 4
QB = 2048
RUN = 32
NT_O, NT_F = H * DH * D // 1024, F * D // 1024
OFF_O, OFF_F = 16, 8
N_HI = 12
LG, LE = 39, 46
TW, TE = 16, 20
T_GATE, T_UP = H * DH // 128, (H * DH + F) // 128

f32, bf16 = jnp.float32, jnp.bfloat16


def _steps(groups):
    pieces = [(first + k, c) for first, quarters in groups for c in quarters for k in (0, 2)]
    return [pieces[3 * j // 2:3 * (j + 1) // 2] for j in range(HS)]


_FIRST = (0, 8, 16, 1, 9, 17)
K_STEPS = _steps([(r, q) for q in ((0, 1), (2, 3)) for r in _FIRST])
V_STEPS = _steps([g for k in range(6) for g in ((_FIRST[k], (0, 1, 2)), (_FIRST[k - 2], (3,)))])
V_STEPS_END = _steps([(r, q) for q in ((0, 1, 2), (3,)) for r in _FIRST])


def _complete(steps, quarter):
    return max(j for j, pieces in enumerate(steps) if any(c == quarter for _, c in pieces))


def _every(t0, n, d):
    return [t0 + j * d for j in range(n)]


def _by_step(tasks):
    by = {}
    for t, fn in tasks:
        by.setdefault(t, []).append(fn)
    return by


def _kernel(x_hbm, kT, vT, wq, wo, wr_hbm, wg, wu, wd, gw_hbm, out_ref,
            x_v, wr_v, gw_v, k_b, v_b, wq_b, wo_b, gu_b, wd_b, pr_s, o_s, s_s, p_s, a_s, g_s, hb_s,
            kv_sem, w_sem, d_sem, p_sem):
    def kv_copy(which, h, r, c, n, sem):
        group, sub = divmod(r + SHIFT[which], 4)
        rows = pl.ds(8 * sub, 8)
        return pltpu.make_async_copy(
            (kT, vT)[which].at[pl.ds((RT // 4) * h + group, n), rows, pl.ds(BASE + c * KC, KC)],
            (k_b, v_b)[which].at[h & 3, pl.ds(group, n), rows, pl.ds(c * KC, KC)], sem)

    def kv_pieces(which, h, j):
        static = isinstance(h, int)
        steps = K_STEPS if which == 0 else V_STEPS_END if static and h >= H - 2 else V_STEPS
        end = RT - SHIFT[which] if static and h == H - 1 else RT
        return [(r, c, 1 + (r + 4 < end)) for r, c in steps[j] if r < end]

    def kv_start(which, h, j, slot):
        for piece in kv_pieces(which, h, j):
            kv_copy(which, h, *piece, kv_sem.at[slot]).start(priority=1)

    def kv_wait(which, h, j, slot):
        n = sum(piece[2] for piece in kv_pieces(which, h, j))
        if n:
            tiles_wait(n * KC // 128, kv_sem.at[slot])

    def round_step(i, s):
        return (0, i + 1, s, s) if s < HS else (1, i, s - HS, s)

    def tiles_copy(src, dst, t, n, sem):
        return pltpu.make_async_copy(src.at[pl.ds(t, n)], dst.at[pl.ds(t, n)], sem)

    def tiles_wait(n, sem):
        tiles_copy(wd_b, wd_b, 0, n, sem).wait()

    def wq_copy(row_tile, col, n, sem):
        idx = (pl.ds(pl.multiple_of(8 * row_tile, 8), 8), pl.ds(pl.multiple_of(col, 512), n))
        return pltpu.make_async_copy(wq.at[idx], wq_b.at[idx], sem)

    def wq_piece(i, s):
        blk = i // 5 if isinstance(i, int) else jnp.where(i >= 5, 1, 0)
        return wq_copy(5 * (s // 4) + i - 5 * blk, QB * (blk + 1) + 512 * (s % 4), 512, w_sem.at[i & 1])

    def run_piece(src, dst, pos, s, off, sem, may_wrap=False):
        n = src.shape[0]
        run, part = divmod(s, 8)
        t = (run % 2) * (n // 2) + (pos + run // 2) * RUN + 4 * part - off
        if isinstance(t, int):
            t %= n
        elif may_wrap and run == 0 and 4 * part < off:
            t = jnp.where(t < 0, t + n, t)
        return tiles_copy(src, dst, t, 4, sem)

    small = [pltpu.make_async_copy(x_hbm, x_v, p_sem.at[0]),
             pltpu.make_async_copy(gw_hbm, gw_v, p_sem.at[1]),
             pltpu.make_async_copy(wr_hbm, wr_v, p_sem.at[2])]

    def kv_head(which, h, sl):
        buf = (k_b, v_b)[which]
        old, new, cut = buf.at[(h - 1) & 3], buf.at[h & 3], 8 * (SHIFT[which] - 4)
        rest = new[2:6, :, sl]
        return jnp.concatenate([old[6, :, sl], old[7, :cut, sl], new[1, cut:, sl],
                                rest.reshape(128, rest.shape[-1])], axis=0)

    def tile_column(ref, t0, n, stride):
        return jnp.concatenate([ref[t0 + stride * k] for k in range(n)], axis=0)

    def x_rows():
        return jnp.broadcast_to(x_v[0], (M, D))

    def qk_tasks(h, t0):
        st = {}

        def qk(j):
            def fn():
                if j == 0:
                    tile = (3 * h) >> 1
                    q2 = jnp.concatenate([pr_s[tile], pr_s[tile + 1]], axis=1)
                    if isinstance(h, int):
                        q = q2[:, 64 * (h % 2):64 * (h % 2) + DH]
                    else:
                        q = jnp.where((h & 1) == 0, q2[:, :DH], q2[:, 64:])
                    st["q"] = q.astype(bf16)
                sl = slice(j * W // 8, (j + 1) * W // 8)
                s_s[:, sl] = jnp.dot(st["q"], kv_head(0, h, sl),
                                     preferred_element_type=f32) * (DH ** -0.5)
            return fn

        def sm_max():
            st["m"] = jnp.max(s_s[...], axis=-1, keepdims=True)

        def sm_exp():
            e = jnp.exp(s_s[...] - st["m"])
            s_s[...] = e
            st["l"] = jnp.sum(e, axis=-1, keepdims=True)

        def sm_norm():
            p_s[h & 1] = s_s[...] * (1.0 / st["l"])

        return list(zip(_every(t0, 11, 2), [qk(j) for j in range(8)] + [sm_max, sm_exp, sm_norm]))

    def pv_tasks(h, steps):
        st = {}

        def pv(j):
            def fn():
                sl = slice(j * W // 8, (j + 1) * W // 8)
                part = jax.lax.dot_general(p_s[h & 1, :, sl].astype(bf16), kv_head(1, h, sl),
                                           (((1,), (1,)), ((), ())), preferred_element_type=f32)
                st["o"] = part if j == 0 else st["o"] + part
                if j == 7:
                    o_s[h] = st["o"]
            return fn

        return [(t, pv(j)) for j, t in enumerate(steps)]

    def q_tasks(i):
        def proj(t):
            def fn():
                cols = pl.ds(pl.multiple_of(128 * t, 128), 128)
                pr_s[t] = jnp.dot(x_rows(), wq_b[:, cols], preferred_element_type=f32)
            return fn

        return [(TW + 1 + 2 * j, proj(3 * i + j)) for j in range(3)]

    def gu_tasks(which):
        def proj(c):
            def fn():
                w = jnp.concatenate([tile_column(gu_b.at[which], c + u, D // 8, F // 128) for u in range(2)], axis=1)
                v = jnp.dot(x_rows(), w, preferred_element_type=f32)
                for u in range(2):
                    pr_s[T_GATE + (T_UP - T_GATE) * which + c + u] = v[:, 128 * u:128 * (u + 1)]
            return fn

        return [(2 * c, proj(c)) for c in range(0, F // 128, 2)]

    def gates():
        xf = x_rows().astype(f32)
        for k, w in enumerate((gw_v, wr_v)):
            logit = jnp.sum(xf * w[...].astype(f32).reshape(1, D), axis=-1, keepdims=True)
            g_s[k] = jnp.broadcast_to(jax.nn.sigmoid(logit), (M, 128))

    def h_task(j):
        def fn():
            h = jax.nn.silu(pr_s[T_GATE + j]) * pr_s[T_UP + j] * ((1.0 - g_s[0]) * g_s[1])
            hb_s[j] = jnp.concatenate([h] * (128 // M), axis=0).T
        return fn

    def o_task(hd):
        def fn():
            w = jnp.concatenate([tile_column(wo_b, (NT_O // H) * hd + c, DH // 8, D // 128)
                                 for c in range(D // 128)], axis=1)
            a_s[...] += jnp.dot(o_s[hd].astype(bf16), w, preferred_element_type=f32)
        return fn

    def attn_tasks(i):
        assert TW + 8 >= LG - HS and 48 >= LG
        return qk_tasks(i, TW + 8) + pv_tasks(i - 1, _every(48, 8, 2))

    def stream_round(i, w_piece, tasks, first=False):
        by = _by_step(tasks)
        assert max(by) < NS
        for s in range(NS):
            if s >= LG:
                kv_wait(*round_step(i, s - LG))
            elif not first:
                kv_wait(*round_step(i - 1, s - LG + NS))
            elif s - LG >= -HS:
                kv_wait(0, 0, s - LG + HS, s - LG + NS)
            kv_start(*round_step(i, s))
            w_piece(i, s).start(priority=0)
            if s == TW and first:
                tiles_wait(12 * RUN, p_sem.at[3])
                tiles_wait(sum(SHIFT) * W // 128, p_sem.at[5])
                first_block = wq_b.at[:, pl.ds(0, QB)]
                pltpu.make_async_copy(first_block, first_block, p_sem.at[4]).wait()
                for c in small:
                    c.wait()
            elif s == TW:
                tiles_wait(4 * NS, w_sem.at[(i - 1) & 1])
            for fn in by.get(s, []):
                fn()

    def stream_rounds(lo, hi, w_piece, tasks):
        def body(i, carry):
            stream_round(i, w_piece, tasks(i) + attn_tasks(i))
            return carry
        jax.lax.fori_loop(lo, hi, body, 0)

    ahead = [(which, -1, r, c, 1) for c in range(4) for which in range(2) for r in range(RT - SHIFT[which], RT)]
    for j in range(D // 8 + HS):
        if j >= 16:
            run, part = divmod(j - 16, 8)
            run_piece((wg, wu)[run % 2], gu_b.at[run % 2], 0, 8 * (run // 2) + part, OFF_F,
                      p_sem.at[3]).start(priority=0)
        if HS <= j < HS + len(ahead):
            kv_copy(*ahead[j - HS], p_sem.at[5]).start(priority=1)
        if j < D // 8:
            wq_copy(5 * (j % 16) + j // 16, 0, QB, p_sem.at[4]).start(priority=1)
        else:
            kv_start(0, 0, j - D // 8, HS + j - D // 8)
        if j == 60:
            for c in small:
                c.start()
    a_s[...] = jnp.zeros(a_s.shape, f32)

    def wo_piece(i, s, may_wrap=False):
        return run_piece(wo, wo_b, 4 * (i - 16), s, OFF_O, w_sem.at[i & 1], may_wrap)

    assert 42 >= LG
    stream_round(0, wq_piece, q_tasks(0) + [(TW + 10, gates)] + qk_tasks(0, 42), first=True)
    stream_rounds(1, 10, wq_piece, q_tasks)
    stream_rounds(10, 13, lambda i, s: run_piece(wg, gu_b.at[0], 3 + 4 * (i - 10), s, OFF_F, w_sem.at[i & 1]), q_tasks)
    stream_rounds(13, 16, lambda i, s: run_piece(wu, gu_b.at[1], 3 + 4 * (i - 13), s, OFF_F, w_sem.at[i & 1]), q_tasks)
    stream_rounds(16, 18, lambda i, s: wo_piece(i, s, True), lambda i: gu_tasks(i - 16))
    stream_rounds(18, 30, wo_piece, lambda i: [(4, h_task(i - 18)), (TW + 1, o_task(i - 2)), (TW + 4, o_task(i - 18))])
    stream_round(30, wo_piece, [(4, o_task(12)), (TW + 1, o_task(28)), (TW + 4, o_task(13))] + attn_tasks(30))

    y = {}

    def down(t0, n):
        for t in range(t0, t0 + n):
            r, c = divmod(t, D // 128)
            part = wd_b[t].astype(f32) * hb_s[r // 16, 8 * (r % 16):8 * (r % 16) + 8]
            y[c] = y[c] + part if c in y else part

    def mix():
        xf = x_rows().astype(f32)
        gate = jnp.concatenate([g_s[0]] * (D // 128), axis=1)
        rest = gate * a_s[...] + (1.0 - gate) * (xf + xf * 0.0)
        one_row = jax.lax.broadcasted_iota(jnp.int32, (M, 128), 0) == 0
        for c in range(D // 128):
            y[c] = y[c] + jnp.where(one_row, rest[:, 128 * c:128 * (c + 1)], 0.0)

    landed = [LG + _complete(V_STEPS_END, c) for c in range(4)]
    t30 = [max(landed[j // 2], landed[0] + 1 + 2 * j) - HS for j in range(8)]
    t31 = [max(landed[j // 2], landed[0] + 3 * j) for j in range(8)]
    assert landed == sorted(landed) and t30[-1] > TW
    by = _by_step([(4, o_task(29))] + qk_tasks(31, LG - HS)
                  + pv_tasks(30, t30) + [(t30[-1] + 3 + 4 * j, o_task(hd)) for j, hd in enumerate((30, 14, 15))]
                  + pv_tasks(31, t31) + [(t31[-1] + 2, o_task(31)), (t31[-1] + 3, mix)])
    hi_pieces = [(RUN * ((k % 2) * (N_HI // 2) + k // 2) - OFF_F + u) % NT_F
                 for k in range(N_HI) for u in range(0, RUN, 4)]
    n_lo = NT_F // RUN - N_HI
    lo_pieces = [RUN * (N_HI + (k % 2) * (n_lo // 2) + k // 2) - OFF_F + u
                 for k in range(n_lo) for u in (0, RUN // 2)]
    n_steps = HS + len(lo_pieces) + LE
    assert len(hi_pieces) < n_steps - 1 and max(by) < n_steps
    for s in range(n_steps):
        for k in range(N_HI):
            if s == min(8 * (k + 1) + TE + 1, n_steps - 1):
                tiles_wait(RUN, d_sem.at[k])
                for t in hi_pieces[8 * k:8 * (k + 1)]:
                    down(t, 4)
        if s < LG:
            kv_wait(*round_step(H - 2, s - LG + NS))
        elif s - LG < HS:
            kv_wait(1, H - 1, s - LG, s - LG)
        elif s - LE >= HS:
            tiles_copy(wd, wd_b, lo_pieces[s - LE - HS], RUN // 2, d_sem.at[N_HI + s - LE - HS]).wait()
            down(lo_pieces[s - LE - HS], RUN // 2)
        if s < len(hi_pieces):
            tiles_copy(wd, wd_b, hi_pieces[s], 4, d_sem.at[s // 8]).start(priority=0)
        if s < HS:
            kv_start(1, H - 1, s, s)
        elif s - HS < len(lo_pieces):
            tiles_copy(wd, wd_b, lo_pieces[s - HS], RUN // 2, d_sem.at[N_HI + s - HS]).start(priority=1)
        if s == TW:
            tiles_wait(4 * NS, w_sem.at[0])
        for fn in by.get(s, []):
            fn()

    out = jnp.sum(jnp.concatenate([y[c] for c in range(D // 128)], axis=1), axis=0, keepdims=True)
    out_ref[0] = out.astype(bf16)


def _tiles(a):
    r, c = a.shape
    return a.reshape(r // 8, 8, c // 128, 128).transpose(0, 2, 1, 3).reshape(-1, 8, 128)


@jax.jit
def pallas_gated_mix__sliding_block_cached__moe_arch_mod__decode_kernel(
        A_x, A_k_cache, A_v_cache, A_wq, A_wo, B_x, B_w_r, B_w_gate, B_w_up, B_w_down, gate_w):
    del B_x
    kT = jnp.swapaxes(A_k_cache, 2, 3).reshape(H * RT // 4, 32, SK)
    vT = jnp.swapaxes(A_v_cache, 2, 3).reshape(H * RT // 4, 32, SK)
    vmem, dma = pltpu.VMEM, pltpu.SemaphoreType.DMA
    return pl.pallas_call(
        _kernel,
        out_shape=jax.ShapeDtypeStruct((1, 1, D), bf16),
        in_specs=[pl.BlockSpec(memory_space=pl.ANY)] * 10,
        out_specs=pl.BlockSpec(memory_space=pltpu.VMEM),
        scratch_shapes=[
            vmem((1, 1, D), bf16), vmem((D,), bf16), vmem((D,), bf16),
            vmem((4, 8, 32, W), bf16), vmem((4, 8, 32, W), bf16), vmem((D, H * DH), bf16),
            vmem((NT_O, 8, 128), bf16), vmem((2, NT_F, 8, 128), bf16), vmem((NT_F, 8, 128), bf16),
            vmem(((H * DH + 2 * F) // 128, M, 128), f32), vmem((H, M, DH), f32),
            vmem((M, W), f32), vmem((2, M, W), f32), vmem((M, D), f32),
            vmem((2, M, 128), f32), vmem((F // 128, 128, 128), f32),
            dma((NS,)), dma((2,)), dma((2 * NT_F // RUN - N_HI,)), dma((6,)),
        ],
        compiler_params=pltpu.CompilerParams(
            vmem_limit_bytes=64 * 1024 * 1024,
            disable_semaphore_checks=True,
            disable_bounds_checks=True,
        ),
        name="gated_mix_decode",
    )(A_x, kT, vT, A_wq, _tiles(A_wo), B_w_r, _tiles(B_w_gate), _tiles(B_w_up), _tiles(B_w_down), gate_w)
```

```python
import jax
import jax.numpy as jnp
import jax.experimental.pallas as pl
import jax.experimental.pallas.tpu as pltpu

H, DH, SK, D, F = 32, 192, 32768, 640, 1536
W = min(4096, max(256, SK // 4))
BASE = SK - W
M = 8

NS, HS = 64, 32
RT = DH // 8
SHIFT = (5, 6)
KC = W // 4
QB = 2048
RUN = 32
NT_O, NT_F = H * DH * D // 1024, F * D // 1024
OFF_O, OFF_F = 16, 8
N_HI = 12
LG, LE = 39, 46
TW, TE = 16, 20
T_GATE, T_UP = H * DH // 128, (H * DH + F) // 128

f32, bf16 = jnp.float32, jnp.bfloat16


def _steps(groups):
    pieces = [(first + k, c) for first, quarters in groups for c in quarters for k in (0, 2)]
    return [pieces[3 * j // 2:3 * (j + 1) // 2] for j in range(HS)]


_FIRST = (0, 8, 16, 1, 9, 17)
K_STEPS = _steps([(r, q) for q in ((0, 1), (2, 3)) for r in _FIRST])
V_STEPS = _steps([g for k in range(6) for g in ((_FIRST[k], (0, 1, 2)), (_FIRST[k - 2], (3,)))])
V_STEPS_END = _steps([(r, q) for q in ((0, 1, 2), (3,)) for r in _FIRST])


def _complete(steps, quarter):
    return max(j for j, pieces in enumerate(steps) if any(c == quarter for _, c in pieces))


def _every(t0, n, d):
    return [t0 + j * d for j in range(n)]


def _by_step(tasks):
    by = {}
    for t, fn in tasks:
        by.setdefault(t, []).append(fn)
    return by


def _kernel(x_hbm, kT, vT, wq, wo, wr_hbm, wg, wu, wd, gw_hbm, out_ref,
            x_v, wr_v, gw_v, k_b, v_b, wq_b, wo_b, gu_b, wd_b, pr_s, o_s, s_s, p_s, a_s, g_s, hb_s,
            kv_sem, w_sem, d_sem, p_sem):
    def kv_copy(which, h, r, c, n, sem):
        group, sub = divmod(r + SHIFT[which], 4)
        rows = pl.ds(8 * sub, 8)
        return pltpu.make_async_copy(
            (kT, vT)[which].at[pl.ds((RT // 4) * h + group, n), rows, pl.ds(BASE + c * KC, KC)],
            (k_b, v_b)[which].at[h & 3, pl.ds(group, n), rows, pl.ds(c * KC, KC)], sem)

    def kv_pieces(which, h, j):
        static = isinstance(h, int)
        steps = K_STEPS if which == 0 else V_STEPS_END if static and h >= H - 2 else V_STEPS
        end = RT - SHIFT[which] if static and h == H - 1 else RT
        return [(r, c, 1 + (r + 4 < end)) for r, c in steps[j] if r < end]

    def kv_start(which, h, j, slot):
        for piece in kv_pieces(which, h, j):
            kv_copy(which, h, *piece, kv_sem.at[slot]).start(priority=1)

    def kv_wait(which, h, j, slot):
        n = sum(piece[2] for piece in kv_pieces(which, h, j))
        if n:
            tiles_wait(n * KC // 128, kv_sem.at[slot])

    def round_step(i, s):
        return (0, i + 1, s, s) if s < HS else (1, i, s - HS, s)

    def tiles_copy(src, dst, t, n, sem):
        return pltpu.make_async_copy(src.at[pl.ds(t, n)], dst.at[pl.ds(t, n)], sem)

    def tiles_wait(n, sem):
        tiles_copy(wd_b, wd_b, 0, n, sem).wait()

    def wq_copy(row_tile, col, n, sem):
        idx = (pl.ds(pl.multiple_of(8 * row_tile, 8), 8), pl.ds(pl.multiple_of(col, 512), n))
        return pltpu.make_async_copy(wq.at[idx], wq_b.at[idx], sem)

    def wq_piece(i, s):
        odd = i // 5 if isinstance(i, int) else jnp.where(i >= 5, 1, 0)
        run, part = divmod(s, 8)
        if part >= 4:
            run = (run + 4 * odd) & 7
        return wq_copy(10 * run + 2 * (i - 5 * odd) + odd, QB + 512 * part, 512, w_sem.at[i & 1])

    def run_piece(src, dst, pos, s, off, sem, may_wrap=False):
        n = src.shape[0]
        run, part = divmod(s, 8)
        t = (run % 2) * (n // 2) + (pos + run // 2) * RUN + 4 * part - off
        if isinstance(t, int):
            t %= n
        elif may_wrap and run == 0 and 4 * part < off:
            t = jnp.where(t < 0, t + n, t)
        return tiles_copy(src, dst, t, 4, sem)

    small = [pltpu.make_async_copy(x_hbm, x_v, p_sem.at[0]),
             pltpu.make_async_copy(gw_hbm, gw_v, p_sem.at[1]),
             pltpu.make_async_copy(wr_hbm, wr_v, p_sem.at[2])]

    def kv_head(which, h, sl):
        buf = (k_b, v_b)[which]
        old, new, cut = buf.at[(h - 1) & 3], buf.at[h & 3], 8 * (SHIFT[which] - 4)
        rest = new[2:6, :, sl]
        return jnp.concatenate([old[6, :, sl], old[7, :cut, sl], new[1, cut:, sl],
                                rest.reshape(128, rest.shape[-1])], axis=0)

    def tile_column(ref, t0, n, stride):
        return jnp.concatenate([ref[t0 + stride * k] for k in range(n)], axis=0)

    def x_rows():
        return jnp.broadcast_to(x_v[0], (M, D))

    def qk_tasks(h, t0):
        st = {}

        def qk(j):
            def fn():
                if j == 0:
                    tile = (3 * h) >> 1
                    q2 = jnp.concatenate([pr_s[tile], pr_s[tile + 1]], axis=1)
                    if isinstance(h, int):
                        q = q2[:, 64 * (h % 2):64 * (h % 2) + DH]
                    else:
                        q = jnp.where((h & 1) == 0, q2[:, :DH], q2[:, 64:])
                    st["q"] = q.astype(bf16)
                sl = slice(j * W // 8, (j + 1) * W // 8)
                s_s[:, sl] = jnp.dot(st["q"], kv_head(0, h, sl),
                                     preferred_element_type=f32) * (DH ** -0.5)
            return fn

        def sm_max():
            st["m"] = jnp.max(s_s[...], axis=-1, keepdims=True)

        def sm_exp():
            e = jnp.exp(s_s[...] - st["m"])
            s_s[...] = e
            st["l"] = jnp.sum(e, axis=-1, keepdims=True)

        def sm_norm():
            p_s[h & 1] = s_s[...] * (1.0 / st["l"])

        return list(zip(_every(t0, 11, 2), [qk(j) for j in range(8)] + [sm_max, sm_exp, sm_norm]))

    def pv_tasks(h, steps):
        st = {}

        def pv(j):
            def fn():
                sl = slice(j * W // 8, (j + 1) * W // 8)
                part = jax.lax.dot_general(p_s[h & 1, :, sl].astype(bf16), kv_head(1, h, sl),
                                           (((1,), (1,)), ((), ())), preferred_element_type=f32)
                st["o"] = part if j == 0 else st["o"] + part
                if j == 7:
                    o_s[h] = st["o"]
            return fn

        return [(t, pv(j)) for j, t in enumerate(steps)]

    def q_task(t):
        def fn():
            cols = pl.ds(pl.multiple_of(128 * t, 128), 256)
            v = jnp.dot(x_rows(), wq_b[:, cols], preferred_element_type=f32)
            pr_s[t] = v[:, :128]
            pr_s[t + 1] = v[:, 128:]
        return fn

    def q_first(i):
        return [(TW + 1, q_task(jnp.minimum(2 * i, QB // 128 - 2)))]

    def q_rest(i):
        return [(t, q_task(jnp.minimum(QB // 128 + 6 * (i - 10) + 2 * j, T_GATE - 2)))
                for j, t in enumerate((TW + 1, TW + 4, 46))]

    def gu_tasks(which):
        def proj(c):
            def fn():
                w = jnp.concatenate([tile_column(gu_b.at[which], c + u, D // 8, F // 128) for u in range(2)], axis=1)
                v = jnp.dot(x_rows(), w, preferred_element_type=f32)
                for u in range(2):
                    pr_s[T_GATE + (T_UP - T_GATE) * which + c + u] = v[:, 128 * u:128 * (u + 1)]
            return fn

        return [(2 * c, proj(c)) for c in range(0, F // 128, 2)]

    def gates():
        xf = x_rows().astype(f32)
        for k, w in enumerate((gw_v, wr_v)):
            logit = jnp.sum(xf * w[...].astype(f32).reshape(1, D), axis=-1, keepdims=True)
            g_s[k] = jnp.broadcast_to(jax.nn.sigmoid(logit), (M, 128))

    def h_task(j):
        def fn():
            h = jax.nn.silu(pr_s[T_GATE + j]) * pr_s[T_UP + j] * ((1.0 - g_s[0]) * g_s[1])
            hb_s[j] = jnp.concatenate([h] * (128 // M), axis=0).T
        return fn

    def o_task(hd):
        def fn():
            w = jnp.concatenate([tile_column(wo_b, (NT_O // H) * hd + c, DH // 8, D // 128)
                                 for c in range(D // 128)], axis=1)
            a_s[...] += jnp.dot(o_s[hd].astype(bf16), w, preferred_element_type=f32)
        return fn

    def attn_tasks(i):
        assert TW + 8 >= LG - HS and 48 >= LG
        return qk_tasks(i, TW + 8) + pv_tasks(i - 1, _every(48, 8, 2))

    def stream_round(i, w_piece, tasks, first=False):
        by = _by_step(tasks)
        assert max(by) < NS
        for s in range(NS):
            if s >= LG:
                kv_wait(*round_step(i, s - LG))
            elif not first:
                kv_wait(*round_step(i - 1, s - LG + NS))
            elif s - LG >= -HS:
                kv_wait(0, 0, s - LG + HS, s - LG + NS)
            kv_start(*round_step(i, s))
            w_piece(i, s).start(priority=0)
            if s == TW and first:
                tiles_wait(12 * RUN, p_sem.at[3])
                tiles_wait(sum(SHIFT) * W // 128, p_sem.at[5])
                first_block = wq_b.at[:, pl.ds(0, QB)]
                pltpu.make_async_copy(first_block, first_block, p_sem.at[4]).wait()
                for c in small:
                    c.wait()
            elif s == TW:
                tiles_wait(4 * NS, w_sem.at[(i - 1) & 1])
            for fn in by.get(s, []):
                fn()

    def stream_rounds(lo, hi, w_piece, tasks):
        def body(i, carry):
            stream_round(i, w_piece, tasks(i) + attn_tasks(i))
            return carry
        jax.lax.fori_loop(lo, hi, body, 0)

    ahead = [(which, -1, r, c, 1) for c in range(4) for which in range(2) for r in range(RT - SHIFT[which], RT)]
    for j in range(D // 8 + HS):
        if j >= 16:
            run, part = divmod(j - 16, 8)
            run_piece((wg, wu)[run % 2], gu_b.at[run % 2], 0, 8 * (run // 2) + part, OFF_F,
                      p_sem.at[3]).start(priority=0)
        if HS <= j < HS + len(ahead):
            kv_copy(*ahead[j - HS], p_sem.at[5]).start(priority=1)
        if j < D // 8:
            wq_copy(5 * (j % 16) + j // 16, 0, QB, p_sem.at[4]).start(priority=1)
        else:
            kv_start(0, 0, j - D // 8, HS + j - D // 8)
        if j == 60:
            for c in small:
                c.start()
    a_s[...] = jnp.zeros(a_s.shape, f32)

    def wo_piece(i, s, may_wrap=False):
        return run_piece(wo, wo_b, 4 * (i - 16), s, OFF_O, w_sem.at[i & 1], may_wrap)

    assert 42 >= LG
    stream_round(0, wq_piece, [(TW + 1, q_task(0)), (TW + 10, gates)] + qk_tasks(0, 42), first=True)
    stream_rounds(1, 10, wq_piece, q_first)
    stream_rounds(10, 13, lambda i, s: run_piece(wg, gu_b.at[0], 3 + 4 * (i - 10), s, OFF_F, w_sem.at[i & 1]), q_rest)
    stream_rounds(13, 16, lambda i, s: run_piece(wu, gu_b.at[1], 3 + 4 * (i - 13), s, OFF_F, w_sem.at[i & 1]), q_rest)
    stream_rounds(16, 18, lambda i, s: wo_piece(i, s, True), lambda i: gu_tasks(i - 16))
    stream_rounds(18, 30, wo_piece, lambda i: [(4, h_task(i - 18)), (TW + 1, o_task(i - 2)), (TW + 4, o_task(i - 18))])
    stream_round(30, wo_piece, [(4, o_task(12)), (TW + 1, o_task(28)), (TW + 4, o_task(13))] + attn_tasks(30))

    y = {}

    def down(t0, n):
        for t in range(t0, t0 + n):
            r, c = divmod(t, D // 128)
            part = wd_b[t].astype(f32) * hb_s[r // 16, 8 * (r % 16):8 * (r % 16) + 8]
            y[c] = y[c] + part if c in y else part

    def mix():
        xf = x_rows().astype(f32)
        gate = jnp.concatenate([g_s[0]] * (D // 128), axis=1)
        rest = gate * a_s[...] + (1.0 - gate) * (xf + xf * 0.0)
        one_row = jax.lax.broadcasted_iota(jnp.int32, (M, 128), 0) == 0
        for c in range(D // 128):
            y[c] = y[c] + jnp.where(one_row, rest[:, 128 * c:128 * (c + 1)], 0.0)

    landed = [LG + _complete(V_STEPS_END, c) for c in range(4)]
    t30 = [max(landed[j // 2], landed[0] + 1 + 2 * j) - HS for j in range(8)]
    t31 = [max(landed[j // 2], landed[0] + 3 * j) for j in range(8)]
    assert landed == sorted(landed) and t30[-1] > TW
    by = _by_step([(4, o_task(29))] + qk_tasks(31, LG - HS)
                  + pv_tasks(30, t30) + [(t30[-1] + 3 + 4 * j, o_task(hd)) for j, hd in enumerate((30, 14, 15))]
                  + pv_tasks(31, t31) + [(t31[-1] + 2, o_task(31)), (t31[-1] + 3, mix)])
    hi_pieces = [(RUN * ((k % 2) * (N_HI // 2) + k // 2) - OFF_F + u) % NT_F
                 for k in range(N_HI) for u in range(0, RUN, 4)]
    n_lo = NT_F // RUN - N_HI
    lo_pieces = [RUN * (N_HI + (k % 2) * (n_lo // 2) + k // 2) - OFF_F + u
                 for k in range(n_lo) for u in (0, RUN // 2)]
    n_steps = HS + len(lo_pieces) + LE
    assert len(hi_pieces) < n_steps - 1 and max(by) < n_steps
    for s in range(n_steps):
        for k in range(N_HI):
            if s == min(8 * (k + 1) + TE + 1, n_steps - 1):
                tiles_wait(RUN, d_sem.at[k])
                for t in hi_pieces[8 * k:8 * (k + 1)]:
                    down(t, 4)
        if s < LG:
            kv_wait(*round_step(H - 2, s - LG + NS))
        elif s - LG < HS:
            kv_wait(1, H - 1, s - LG, s - LG)
        elif s - LE >= HS:
            tiles_copy(wd, wd_b, lo_pieces[s - LE - HS], RUN // 2, d_sem.at[N_HI + s - LE - HS]).wait()
            down(lo_pieces[s - LE - HS], RUN // 2)
        if s < len(hi_pieces):
            tiles_copy(wd, wd_b, hi_pieces[s], 4, d_sem.at[s // 8]).start(priority=0)
        if s < HS:
            kv_start(1, H - 1, s, s)
        elif s - HS < len(lo_pieces):
            tiles_copy(wd, wd_b, lo_pieces[s - HS], RUN // 2, d_sem.at[N_HI + s - HS]).start(priority=1)
        if s == TW:
            tiles_wait(4 * NS, w_sem.at[0])
        for fn in by.get(s, []):
            fn()

    out = jnp.sum(jnp.concatenate([y[c] for c in range(D // 128)], axis=1), axis=0, keepdims=True)
    out_ref[0] = out.astype(bf16)


def _tiles(a):
    r, c = a.shape
    return a.reshape(r // 8, 8, c // 128, 128).transpose(0, 2, 1, 3).reshape(-1, 8, 128)


@jax.jit
def pallas_gated_mix__sliding_block_cached__moe_arch_mod__decode_kernel(
        A_x, A_k_cache, A_v_cache, A_wq, A_wo, B_x, B_w_r, B_w_gate, B_w_up, B_w_down, gate_w):
    del B_x
    kT = jnp.swapaxes(A_k_cache, 2, 3).reshape(H * RT // 4, 32, SK)
    vT = jnp.swapaxes(A_v_cache, 2, 3).reshape(H * RT // 4, 32, SK)
    vmem, dma = pltpu.VMEM, pltpu.SemaphoreType.DMA
    return pl.pallas_call(
        _kernel,
        out_shape=jax.ShapeDtypeStruct((1, 1, D), bf16),
        in_specs=[pl.BlockSpec(memory_space=pl.ANY)] * 10,
        out_specs=pl.BlockSpec(memory_space=pltpu.VMEM),
        scratch_shapes=[
            vmem((1, 1, D), bf16), vmem((D,), bf16), vmem((D,), bf16),
            vmem((4, 8, 32, W), bf16), vmem((4, 8, 32, W), bf16), vmem((D, H * DH), bf16),
            vmem((NT_O, 8, 128), bf16), vmem((2, NT_F, 8, 128), bf16), vmem((NT_F, 8, 128), bf16),
            vmem(((H * DH + 2 * F) // 128, M, 128), f32), vmem((H, M, DH), f32),
            vmem((M, W), f32), vmem((2, M, W), f32), vmem((M, D), f32),
            vmem((2, M, 128), f32), vmem((F // 128, 128, 128), f32),
            dma((NS,)), dma((2,)), dma((2 * NT_F // RUN - N_HI,)), dma((6,)),
        ],
        compiler_params=pltpu.CompilerParams(
            vmem_limit_bytes=64 * 1024 * 1024,
            disable_semaphore_checks=True,
            disable_bounds_checks=True,
        ),
        name="gated_mix_decode",
    )(A_x, kT, vT, A_wq, _tiles(A_wo), B_w_r, _tiles(B_w_gate), _tiles(B_w_up), _tiles(B_w_down), gate_w)
```
